```python
import jax
import jax.numpy as jnp

def _softmax(x, axis=-1):
    return jax.nn.softmax(x, axis=axis)

def _gelu(x):
    return jax.nn.gelu(x, approximate=True)

def _silu(x):
    return jax.nn.silu(x)

def _sigmoid(x):
    return jax.nn.sigmoid(x)

def _layernorm(x, axis=-1, eps=1e-05):
    m = jnp.mean(x, axis=axis, keepdims=True)
    v = jnp.var(x, axis=axis, keepdims=True)
    return (x - m) / jnp.sqrt(v + eps)

def _scatter_add(tgt, idx, src, axis=0):
    return tgt.at[idx].add(src)

def _segment_sum(src, seg, n):
    return jax.ops.segment_sum(src, seg, n)

class _Rng:

    def __init__(self, key):
        self._k = key

    def _next(self):
        self._k, sub = jax.random.split(self._k)
        return sub

    def normal(self, shape):
        return jax.random.normal(self._next(), shape, dtype=jnp.bfloat16)

    def randint(self, lo, hi, shape):
        return jax.random.randint(self._next(), shape, lo, hi, dtype=jnp.int32)

    def uniform(self, shape, lo=0.0, hi=1.0):
        return jax.random.uniform(self._next(), shape, jnp.bfloat16, lo, hi)

    def permutation(self, n):
        return jax.random.permutation(self._next(), n)
kernel_name = 'gated_mix__memory_aug_recurrent_mem_tr__moe_arch_mod__prompt'

def setup_inputs():
    _rng = _Rng(jax.random.key(int.from_bytes(__import__("os").urandom(4), "little")))
    _w = lambda a: (lambda t: t.astype(jnp.bfloat16) if jnp.issubdtype(t.dtype, jnp.floating) else t)(jnp.asarray(a))

    def _A_setup():
        B, S, Dm = (1, 2048, 1024)
        H, Dh = (32, 128)
        M, seg = (8, 32)
        seg = min(seg, S)
        S = S // seg * seg
        return {'x': _w((lambda *s: _rng.normal(s) * 0.05)(B, S, Dm)), 'mem0': _w((lambda *s: _rng.normal(s) * 0.05)(B, M, Dm)), 'Wq': _w((lambda *s: _rng.normal(s) * 0.05)(Dm, H, Dh) * Dm ** (-0.5)), 'Wk': _w((lambda *s: _rng.normal(s) * 0.05)(Dm, H, Dh) * Dm ** (-0.5)), 'Wv': _w((lambda *s: _rng.normal(s) * 0.05)(Dm, H, Dh) * Dm ** (-0.5)), 'Wo': _w((lambda *s: _rng.normal(s) * 0.05)(H, Dh, Dm) * (H * Dh) ** (-0.5)), 'seg_len': seg}
    _A_in = _A_setup()

    def _B_setup():
        B, S, D, F, C = (1, 2048, 1024, 3584, 8)
        return {'x': _w((lambda *s: _rng.normal(s) * 0.05)(B, S, D)), 'w_r': _w((lambda *s: _rng.normal(s) * 0.05)(D)), 'w_gate': _w((lambda *s: _rng.normal(s) * 0.05)(D, F)), 'w_up': _w((lambda *s: _rng.normal(s) * 0.05)(D, F)), 'w_down': _w((lambda *s: _rng.normal(s) * 0.05)(F, D))}
    _B_in = _B_setup()
    return {'A_x': _A_in['x'], 'A_mem0': _A_in['mem0'], 'A_Wq': _A_in['Wq'], 'A_Wk': _A_in['Wk'], 'A_Wv': _A_in['Wv'], 'A_Wo': _A_in['Wo'], 'A_seg_len': _A_in['seg_len'], 'B_x': _B_in['x'], 'B_w_r': _B_in['w_r'], 'B_w_gate': _B_in['w_gate'], 'B_w_up': _B_in['w_up'], 'B_w_down': _B_in['w_down'], 'gate_w': _w((lambda *s: _rng.normal(s) * 0.05)(1024))}

def reference(A_x, A_mem0, A_Wq, A_Wk, A_Wv, A_Wo, A_seg_len, B_x, B_w_r, B_w_gate, B_w_up, B_w_down, gate_w):

    def _A_ref(x, mem0, Wq, Wk, Wv, Wo, seg_len):
        B, S, Dm = x.shape
        H, Dh = (Wq.shape[1], Wq.shape[2])
        M = mem0.shape[1]
        scale = Dh ** (-0.5)
        n_seg = S // seg_len
        L = M + seg_len
        idx = jnp.arange(L)
        mask = (idx[:, None] < M) | (idx[:, None] >= idx[None, :])
        mem = mem0
        outs = []
        for s in range(n_seg):
            xs = x[:, s * seg_len:(s + 1) * seg_len, :].copy()
            h = jnp.concatenate([mem, xs], axis=1)
            q = jnp.einsum('btd,dhe->bhte', h, Wq)
            k = jnp.einsum('btd,dhe->bhte', h, Wk)
            v = jnp.einsum('btd,dhe->bhte', h, Wv)
            scores = jnp.einsum('bhqe,bhke->bhqk', q, k) * scale
            scores = jnp.where(mask[None, None], scores, -1000000000.0)
            p = _softmax(scores, axis=-1)
            o = jnp.einsum('bhqk,bhke->bhqe', p, v)
            o = jnp.einsum('bhte,hed->btd', o, Wo)
            mem = o[:, :M, :].copy()
            outs.append(o[:, M:, :])
        return jnp.concatenate(outs, axis=1)

    def _B_ref(x, w_r, w_gate, w_up, w_down):
        B, S, D = x.shape
        C = 8
        r = x @ w_r
        idx = jnp.argsort(-r, axis=-1)[:, :C]
        idx_e = jnp.repeat(idx.reshape(B, C, 1), D, axis=2)
        x_sel = jnp.take_along_axis(x, idx_e, axis=1)
        g = _silu(x_sel @ w_gate)
        u = x_sel @ w_up
        y = g * u @ w_down
        r_sel = _sigmoid(jnp.take_along_axis(r, idx, axis=1))
        y = y * r_sel.reshape(B, C, 1)
        b_off = (jnp.arange(B) * S).reshape(B, 1)
        flat_idx = (idx + b_off).reshape(B * C)
        zero = (x * 0.0).reshape(B * S, D)
        upd = _scatter_add(zero, flat_idx, y.reshape(B * C, D), axis=0)
        return x + upd.reshape(B, S, D)
    x = A_x
    g = _sigmoid((x * gate_w).sum(-1, keepdims=True))
    a = _A_ref(x, A_mem0, A_Wq, A_Wk, A_Wv, A_Wo, A_seg_len)
    b = _B_ref(x, B_w_r, B_w_gate, B_w_up, B_w_down)
    return g * a + (1 - g) * b
```

```python
import functools

import jax
import jax.numpy as jnp
from jax import lax
import jax.experimental.pallas as pl
import jax.experimental.pallas.tpu as pltpu

_LANES = 128
_TOP_C = 8
_MASKED = -1000000000.0
_KEY_BASE = 0x20000000

_BF16 = jnp.bfloat16
_F32 = jnp.float32
_U32 = jnp.uint32
_NT = (((1,), (1,)), ((), ()))


def _as_bf16(words):
    return pltpu.bitcast(words, _BF16)


def _as_words(rows):
    return pltpu.bitcast(rows, _U32)


def _dot(a, b):
    return jnp.dot(a, b, preferred_element_type=_F32)


def _iota(shape, dim):
    return lax.broadcasted_iota(jnp.int32, shape, dim)


def _kernel(x_hbm, mem0_ref, wq_hbm, wk_hbm, wv_hbm, wo_hbm, wr_ref, gw_ref,
            wg_hbm, wu_hbm, wd_hbm, out_hbm,
            x_buf, x0_buf, wqkv, wo, wg, wu, wd, q_buf, k_buf, v_buf,
            acc_buf, g_buf, out_buf, w_sem, x_sem, wo_sem, ffn_sem, out_sem,
            *, n_seg, n_heads, d_model, d_ff, scale):
    n_pairs = n_heads // 2
    n_blk = d_model // _LANES
    f_blk = d_ff // _LANES
    n_rows0 = n_seg * 8
    seq = n_seg * 32

    def w_copy(m, p):
        src = (wq_hbm, wk_hbm, wv_hbm)[m].bitcast(_U32)
        return pltpu.make_async_copy(src.at[:, :, :, p, :], wqkv.at[m, p], w_sem.at[m, p])

    def col_copy(hbm, dst, j, sem):
        src = hbm.bitcast(_U32).at[:, pl.ds(j * _LANES, _LANES)]
        return pltpu.make_async_copy(src, dst.at[j], sem)

    x0_copy = pltpu.make_async_copy(
        x_hbm.at[:, pl.ds(0, 1)], x_buf.at[:, pl.ds(0, 1)], x_sem.at[0])
    x1_copy = pltpu.make_async_copy(
        x_hbm.at[:, pl.ds(1, 3)], x_buf.at[:, pl.ds(1, 3)], x_sem.at[1])
    wo_copies = [col_copy(wo_hbm, wo, j, wo_sem.at[0]) for j in range(n_blk)]
    ffn_copies = ([col_copy(wg_hbm, wg, j, ffn_sem.at[0]) for j in range(f_blk)]
                  + [col_copy(wu_hbm, wu, j, ffn_sem.at[0]) for j in range(f_blk)]
                  + [col_copy(wd_hbm, wd, j, ffn_sem.at[0]) for j in range(n_blk)])

    ahead = 2
    x0_copy.start()
    for p in range(ahead):
        for m in range(3):
            w_copy(m, p).start()
    x0_copy.wait()
    x0_buf[...] = _as_words(x_buf[:, 0].reshape(n_rows0, d_model))

    def prologue(p, carry):
        @pl.when(p + ahead < n_pairs)
        def _():
            for m in range(3):
                w_copy(m, p + ahead).start()

        @pl.when(p == n_pairs // 2)
        def _():
            x1_copy.start()
            for c in wo_copies:
                c.start()

        for m in range(3):
            w_copy(m, p).wait()
        x0 = _as_bf16(x0_buf[...])
        for m in range(3):
            raw = wqkv[m, p].reshape(d_model, _LANES)
            halves = (raw << 16, raw & jnp.uint32(0xFFFF0000))
            for par in range(2):
                w = pltpu.bitcast(halves[par], _F32).astype(_BF16)
                wqkv[m, p, :, par] = _as_words(w).reshape(d_model // 16, 8, _LANES)
                y = _dot(x0, w)
                h = 2 * p + par
                if m == 0:
                    q_buf[h] = _as_words(y.astype(_BF16))
                else:
                    (k_buf, v_buf)[m - 1][h] = pltpu.bitcast(y, _U32)
        return carry

    lax.fori_loop(0, n_pairs, prologue, 0)

    for c in ffn_copies:
        c.start()
    x1_copy.wait()
    for c in wo_copies:
        c.wait()

    def weight(m, h):
        words = wqkv[m, h // 2, :, h % 2].reshape(d_model // 2, _LANES)
        return _as_bf16(words)

    def out_proj(o, h0, h1, j):
        lhs = jnp.concatenate(o[h0:h1], axis=1)
        return _dot(lhs, _as_bf16(wo[j, h0 * 64:h1 * 64, :]))

    row, col = _iota((32, 48), 0), _iota((32, 48), 1)
    visible = (col < 40) & ((row < 8) | (col <= row + 8))
    hidden = jnp.where(col < 40, _MASKED, -jnp.inf).astype(_F32)
    pad = jnp.zeros((8, _LANES), _F32)
    w_r = wr_ref[...].astype(_F32)
    gate_w = gw_ref[...].astype(_F32)
    lane = _iota((8, _LANES), 1)
    n_keys = seq // (8 * _LANES)

    def row_dot(xs, w):
        t = xs[:, :_LANES] * w[0:1]
        for j in range(1, n_blk):
            t = t + xs[:, j * _LANES:(j + 1) * _LANES] * w[j:j + 1]
        return jnp.sum(t, axis=1, keepdims=True)

    def step(s, carry):
        mem, scores = carry
        xs = x_buf[s].reshape(32, d_model).astype(_F32)
        h = jnp.concatenate([mem, xs[8:]], axis=0).astype(_BF16)
        grp = pl.ds(pl.multiple_of(s * 8, 8), 8)

        def with_first_tokens(buf, hd, y):
            y0 = pltpu.bitcast(buf[hd, grp, :], _F32)
            full = jnp.concatenate([y[:8], y0, y[8:], pad], axis=0).astype(_BF16)
            buf[hd, grp, :] = _as_words(full[:16])
            return full

        q, k, v, e, inv, o = {}, {}, {}, {}, {}, [None] * n_heads

        def project(hd):
            q[hd] = _dot(h, weight(0, hd)).astype(_BF16)
            k[hd] = with_first_tokens(k_buf, hd, _dot(h, weight(1, hd)))
            v[hd] = with_first_tokens(v_buf, hd, _dot(h, weight(2, hd)))

        def attend(hd):
            sc = lax.dot_general(q[hd], k[hd], _NT, preferred_element_type=_F32)
            sc = jnp.where(visible, sc * scale, hidden)
            ex = jnp.exp(sc - jnp.max(sc, axis=1, keepdims=True))
            inv[hd] = 1.0 / jnp.sum(ex, axis=1, keepdims=True)
            e[hd] = ex.astype(_BF16)

        def combine(hd):
            o[hd] = (_dot(e[hd], v[hd]) * inv[hd]).astype(_BF16)

        lag_a, lag_c = 2, 4
        for i in range(0, n_heads, 2):
            project(i)
            project(i + 1)
            for hd in (i - lag_a, i + 1 - lag_a):
                if hd >= 0:
                    attend(hd)
            for hd in (i - lag_c, i + 1 - lag_c):
                if hd >= 0:
                    combine(hd)
        half = n_heads // 2
        part = []
        for j in range(n_blk):
            part.append(out_proj(o, 0, half, j))
            i = n_heads + 2 * (j // 2)
            if j % 2 == 1:
                for hd in (i - lag_a, i + 1 - lag_a):
                    if hd < n_heads:
                        attend(hd)
                for hd in (i - lag_c, i + 1 - lag_c):
                    if hd < n_heads:
                        combine(hd)
        a = jnp.concatenate(
            [part[j] + out_proj(o, half, n_heads, j) for j in range(n_blk)], axis=1)

        g = jax.nn.sigmoid(row_dot(xs, gate_w))
        r = row_dot(xs, w_r)
        rows = pl.ds(pl.multiple_of(s * 32, 32), 32)
        g_buf[rows, :] = jnp.broadcast_to(g, (32, _LANES))
        rest = (1.0 - g) * xs
        acc_buf[rows, :] = jnp.concatenate([rest[:8], g[8:] * a[8:] + rest[8:]], axis=0)
        scores = list(scores)
        for t in range(4):
            for u in range(n_keys):
                scores[u] = jnp.where(
                    lane == 4 * s + t - u * _LANES, r[8 * t:8 * t + 8], scores[u])
        return a[:8], tuple(scores)

    init = tuple(jnp.zeros((8, _LANES), _F32) for _ in range(n_keys))
    _, scores = lax.fori_loop(0, n_seg, step, (mem0_ref[...].astype(_F32), init))

    row, col = _iota((64, _LANES), 0), _iota((64, _LANES), 1)
    own = (row >> 3) == (col >> 4)
    visible0 = own & ((col & 15) <= 8 + (row & 7))
    hidden0 = jnp.where(own, _MASKED, -jnp.inf).astype(_F32)
    n_chunks = n_seg // 8

    def first_tokens(hd, carry):
        ex, inv = [], []
        for c in range(n_chunks):
            q = _as_bf16(q_buf[hd, c * 32:(c + 1) * 32, :])
            k = _as_bf16(k_buf[hd, c * 64:(c + 1) * 64, :])
            sc = lax.dot_general(q, k, _NT, preferred_element_type=_F32)
            sc = jnp.where(visible0, sc * scale, hidden0)
            t = jnp.exp(sc - jnp.max(sc, axis=1, keepdims=True))
            inv.append(1.0 / jnp.sum(t, axis=1, keepdims=True))
            ex.append(t.astype(_BF16))
        for c in range(n_chunks):
            v = _as_bf16(v_buf[hd, c * 64:(c + 1) * 64, :])
            q_buf[hd, c * 32:(c + 1) * 32, :] = _as_words(
                (_dot(ex[c], v) * inv[c]).astype(_BF16))
        return carry

    lax.fori_loop(0, n_heads, first_tokens, 0)

    sub = _iota((8, _LANES), 0)
    keys = []
    for u in range(n_keys):
        r = scores[u].astype(_BF16).astype(_F32)
        bits = lax.shift_right_logical(
            pltpu.bitcast(jnp.where(r == 0.0, 0.0, r), jnp.int32), 16)
        order = jnp.where(bits >= 0x8000, 0xFFFF - bits, bits + 0x8000)
        order = jnp.where(r != r, 0, order)
        token = (lane + u * _LANES) * 8 + sub
        keys.append(pltpu.bitcast(_KEY_BASE + order * seq + (seq - 1 - token), _F32))

    sub_d = _iota((8, d_model), 0)
    picked = jnp.zeros((8, _LANES), jnp.int32)
    x_sel = jnp.zeros((8, d_model), _F32)
    tokens = []
    for i in range(_TOP_C):
        best = functools.reduce(jnp.maximum, keys)
        best = jnp.max(jnp.max(best, axis=1, keepdims=True), axis=0, keepdims=True)
        keys = [jnp.where(kk == best, 0.0, kk) for kk in keys]
        code = pltpu.bitcast(jnp.broadcast_to(best, (8, _LANES)), jnp.int32) - _KEY_BASE
        picked = jnp.where(sub == i, code, picked)
        tok = seq - 1 - (code[0, 0] & (seq - 1))
        tokens.append(tok)
        grp = x_buf[tok >> 5, (tok >> 3) & 3].astype(_F32)
        one = jnp.sum(jnp.where(sub_d == (tok & 7), grp, 0.0), axis=0, keepdims=True)
        x_sel = jnp.where(sub_d == i, one, x_sel)
    order = picked >> (seq.bit_length() - 1)
    bits = jnp.where(order >= 0x8000, order - 0x8000, 0xFFFF - order)
    r_sel = jax.nn.sigmoid(pltpu.bitcast(bits << 16, _F32))

    for c in ffn_copies:
        c.wait()
    xb = x_sel.astype(_BF16)
    hidden_act = []
    for j in range(f_blk):
        gt = _dot(xb, _as_bf16(wg[j]))
        up = _dot(xb, _as_bf16(wu[j]))
        hidden_act.append((gt * jax.nn.sigmoid(gt) * up).astype(_BF16))
    hidden_act = jnp.concatenate(hidden_act, axis=1)
    y = [_dot(hidden_act, _as_bf16(wd[j])) * r_sel for j in range(n_blk)]
    for i, tok in enumerate(tokens):
        at = pl.ds(tok, 1)
        keep = 1.0 - g_buf[at, :]
        acc_buf[at, :] += jnp.concatenate([keep * yj[i:i + 1] for yj in y], axis=1)

    segs = 16
    n_out = n_seg // segs

    def out_copy(c):
        span = pl.ds(c * segs, segs)
        return pltpu.make_async_copy(out_buf.at[span], out_hbm.at[span], out_sem.at[c])

    def finish(c, carry):
        words = pl.ds(pl.multiple_of(c * segs * 4, segs * 4), segs * 4)
        o = jnp.concatenate(
            [_as_bf16(q_buf[hd, words, :]) for hd in range(n_heads)], axis=1)
        a = jnp.concatenate([_dot(o, _as_bf16(wo[j])) for j in range(n_blk)], axis=1)
        for t in range(segs):
            base = pl.multiple_of((c * segs + t) * 32, 32)
            first = acc_buf[pl.ds(base, 8), :] + jnp.tile(
                g_buf[pl.ds(base, 8), :], (1, n_blk)) * a[8 * t:8 * t + 8]
            out_buf[c * segs + t, 0] = first.astype(out_buf.dtype)
            for u in range(1, 4):
                out_buf[c * segs + t, u] = acc_buf[
                    pl.ds(base + 8 * u, 8), :].astype(out_buf.dtype)
        out_copy(c).start()
        return carry

    lax.fori_loop(0, n_out, finish, 0)
    for c in range(n_out):
        out_copy(c).wait()


@functools.partial(jax.jit, static_argnames=("A_seg_len",))
def pallas_gated_mix__memory_aug_recurrent_mem_tr__moe_arch_mod__prompt_kernel(
    A_x, A_mem0, A_Wq, A_Wk, A_Wv, A_Wo, A_seg_len,
    B_x, B_w_r, B_w_gate, B_w_up, B_w_down, gate_w,
):
    del B_x
    batch, seq, d_model = A_x.shape
    _, n_heads, d_head = A_Wq.shape
    d_ff = B_w_gate.shape[1]
    assert batch == 1 and A_seg_len == 32 and A_mem0.shape[1] == 8 and d_head == _LANES
    assert seq % 1024 == 0 and seq & (seq - 1) == 0 and d_model == 8 * _LANES
    n_seg = seq // A_seg_len
    n_blk, f_blk = d_model // _LANES, d_ff // _LANES

    def by_pair(w):
        return w.reshape(d_model // 16, 2, 8, n_heads, d_head)

    hbm = pl.BlockSpec(memory_space=pl.ANY)
    vmem = pl.BlockSpec(memory_space=pltpu.VMEM)
    out = pl.pallas_call(
        functools.partial(_kernel, n_seg=n_seg, n_heads=n_heads, d_model=d_model,
                          d_ff=d_ff, scale=d_head ** -0.5),
        out_shape=jax.ShapeDtypeStruct((n_seg, 4, 8, d_model), A_x.dtype),
        in_specs=[hbm, vmem, hbm, hbm, hbm, hbm, vmem, vmem, hbm, hbm, hbm],
        out_specs=hbm,
        scratch_shapes=[
            pltpu.VMEM((n_seg, 4, 8, d_model), A_x.dtype),
            pltpu.VMEM((n_seg * 4, d_model), _U32),
            pltpu.VMEM((3, n_heads // 2, d_model // 16, 2, 8, _LANES), _U32),
            pltpu.VMEM((n_blk, n_heads * d_head // 2, _LANES), _U32),
            pltpu.VMEM((f_blk, d_model // 2, _LANES), _U32),
            pltpu.VMEM((f_blk, d_model // 2, _LANES), _U32),
            pltpu.VMEM((n_blk, d_ff // 2, _LANES), _U32),
            pltpu.VMEM((n_heads, n_seg * 4, _LANES), _U32),
            pltpu.VMEM((n_heads, n_seg * 8, _LANES), _U32),
            pltpu.VMEM((n_heads, n_seg * 8, _LANES), _U32),
            pltpu.VMEM((seq, d_model), _F32),
            pltpu.VMEM((seq, _LANES), _F32),
            pltpu.VMEM((n_seg, 4, 8, d_model), A_x.dtype),
            pltpu.SemaphoreType.DMA((3, n_heads // 2)),
            pltpu.SemaphoreType.DMA((2,)),
            pltpu.SemaphoreType.DMA((1,)),
            pltpu.SemaphoreType.DMA((1,)),
            pltpu.SemaphoreType.DMA((n_seg // 16,)),
        ],
        compiler_params=pltpu.CompilerParams(vmem_limit_bytes=120 * 2**20),
        name="gated_rmt_mod",
    )(
        A_x.reshape(n_seg, 4, 8, d_model),
        A_mem0.reshape(8, d_model),
        by_pair(A_Wq), by_pair(A_Wk), by_pair(A_Wv),
        A_Wo.reshape(n_heads * d_head, d_model),
        B_w_r.reshape(n_blk, _LANES), gate_w.reshape(n_blk, _LANES),
        B_w_gate, B_w_up, B_w_down,
    )
    return out.reshape(batch, seq, d_model)
```

```python
import functools

import jax
import jax.numpy as jnp
from jax import lax
import jax.experimental.pallas as pl
import jax.experimental.pallas.tpu as pltpu

_LANES = 128
_TOP_C = 8
_MASKED = -1000000000.0
_KEY_BASE = 0x20000000
_FFN_AT = 3
LAG_A, LAG_C = 2, 4
TAIL = {1: (('a', -2), ('a', -1), ('c', -4), ('c', -3)), 6: (('c', -2), ('c', -1))}
SPLIT = 2

_BF16 = jnp.bfloat16
_F32 = jnp.float32
_U32 = jnp.uint32
_NT = (((1,), (1,)), ((), ()))


def _as_bf16(words):
    return pltpu.bitcast(words, _BF16)


def _as_words(rows):
    return pltpu.bitcast(rows, _U32)


def _dot(a, b):
    return jnp.dot(a, b, preferred_element_type=_F32)


def _iota(shape, dim):
    return lax.broadcasted_iota(jnp.int32, shape, dim)


def _kernel(x_hbm, mem0_ref, wq_hbm, wk_hbm, wv_hbm, wo_hbm, wr_ref, gw_ref,
            wg_hbm, wu_hbm, wd_hbm, out_hbm,
            x_buf, x0_buf, wqkv, wo, wg, wu, wd, qkv0, acc_buf, g_buf, r_buf, out_buf,
            w_sem, x0_sem, x_sem, wo_sem, ffn_sem, out_sem,
            *, n_seg, n_heads, d_model, d_ff, scale):
    n_pairs = n_heads // 2
    n_blk = d_model // _LANES
    f_blk = d_ff // _LANES
    n_rows0 = n_seg * 8
    seq = n_seg * 32
    span = n_seg // n_pairs

    def w_copy(m, p):
        src = (wq_hbm, wk_hbm, wv_hbm)[m].bitcast(_U32)
        return pltpu.make_async_copy(src.at[:, :, :, p, :], wqkv.at[m, p], w_sem.at[m, p])

    def col_copy(hbm, dst, j, sem):
        cols = pl.ds(j * _LANES if isinstance(j, int) else pl.multiple_of(j * _LANES, _LANES), _LANES)
        return pltpu.make_async_copy(hbm.bitcast(_U32).at[:, cols], dst.at[j], sem)

    def x_copy(p):
        at = (pl.ds(p * span, span), pl.ds(1, 3))
        return pltpu.make_async_copy(x_hbm.at[at], x_buf.at[at], x_sem.at[p])

    def out_copy(first, count):
        at = pl.ds(first, count)
        return pltpu.make_async_copy(out_buf.at[at], out_hbm.at[at], out_sem.at[0])

    x0_copy = pltpu.make_async_copy(
        x_hbm.at[:, pl.ds(0, 1)], x_buf.at[:, pl.ds(0, 1)], x0_sem.at[0])
    ffn_copies = ([col_copy(wg_hbm, wg, j, ffn_sem.at[0]) for j in range(f_blk)]
                  + [col_copy(wu_hbm, wu, j, ffn_sem.at[0]) for j in range(f_blk)]
                  + [col_copy(wd_hbm, wd, j, ffn_sem.at[0]) for j in range(n_blk)])

    w_r = wr_ref[...].astype(_F32)
    gate_w = gw_ref[...].astype(_F32)
    lane = _iota((8, _LANES), 1)
    n_keys = seq // (8 * _LANES)

    def row_dot(xs, w):
        t = xs[:, :_LANES] * w[0:1]
        for j in range(1, n_blk):
            t = t + xs[:, j * _LANES:(j + 1) * _LANES] * w[j:j + 1]
        return jnp.sum(t, axis=1, keepdims=True)

    def fetch(p):
        for m in range(3):
            w_copy(m, p).start()
        x_copy(p).start()

    x0_copy.start()
    fetch(0)
    x0_copy.wait()
    fetch(1)
    x0_buf[...] = _as_words(x_buf[:, 0].reshape(n_rows0, d_model))

    def prologue(p, scores):
        @pl.when(p + 2 < n_pairs)
        def _():
            fetch(p + 2)

        @pl.when(p >= n_pairs - n_blk)
        def _():
            col_copy(wo_hbm, wo, p - (n_pairs - n_blk), wo_sem.at[0]).start()

        for m in range(3):
            w_copy(m, p).wait()
        x_copy(p).wait()
        x0 = _as_bf16(x0_buf[...])
        for m in range(3):
            raw = wqkv[m, p].reshape(d_model, _LANES)
            halves = (raw << 16, raw & jnp.uint32(0xFFFF0000))
            for par in range(2):
                w = pltpu.bitcast(halves[par], _F32).astype(_BF16)
                wqkv[m, p, :, par] = _as_words(w).reshape(d_model // 16, 8, _LANES)
                qkv0[m, 2 * p + par] = _dot(x0, w)
        scores = list(scores)
        for t in range(span):
            s = p * span + t
            xs = x_buf[s].reshape(32, d_model).astype(_F32)
            g = jax.nn.sigmoid(row_dot(xs, gate_w))
            r = row_dot(xs, w_r)
            rows = pl.ds(pl.multiple_of(s * 32, 32), 32)
            g_buf[rows, :] = jnp.broadcast_to(g, (32, _LANES))
            acc_buf[rows, :] = (1.0 - g) * xs
            for b in range(4):
                for u in range(n_keys):
                    scores[u] = jnp.where(
                        lane == 4 * s + b - u * _LANES, r[8 * b:8 * b + 8], scores[u])
        return tuple(scores)

    init = tuple(jnp.zeros((8, _LANES), _F32) for _ in range(n_keys))
    with jax.named_scope('S_prologue'):
        scores = lax.fori_loop(0, n_pairs, prologue, init)
    for u in range(n_keys):
        r_buf[u] = scores[u]

    for c in ffn_copies:
        c.start()
    for j in range(n_blk):
        col_copy(wo_hbm, wo, j, wo_sem.at[0]).wait()

    def routed_ffn():
        sub = _iota((8, _LANES), 0)
        keys = []
        for u in range(n_keys):
            r = r_buf[u].astype(_BF16).astype(_F32)
            bits = lax.shift_right_logical(
                pltpu.bitcast(jnp.where(r == 0.0, 0.0, r), jnp.int32), 16)
            order = jnp.where(bits >= 0x8000, 0xFFFF - bits, bits + 0x8000)
            order = jnp.where(r != r, 0, order)
            token = (lane + u * _LANES) * 8 + sub
            keys.append(pltpu.bitcast(_KEY_BASE + order * seq + (seq - 1 - token), _F32))

        sub_d = _iota((8, d_model), 0)
        picked = jnp.zeros((8, _LANES), jnp.int32)
        x_sel = jnp.zeros((8, d_model), _F32)
        tokens = []
        for i in range(_TOP_C):
            best = functools.reduce(jnp.maximum, keys)
            best = jnp.max(jnp.max(best, axis=1, keepdims=True), axis=0, keepdims=True)
            keys = [jnp.where(kk == best, 0.0, kk) for kk in keys]
            code = pltpu.bitcast(jnp.broadcast_to(best, (8, _LANES)), jnp.int32) - _KEY_BASE
            picked = jnp.where(sub == i, code, picked)
            tok = seq - 1 - (code[0, 0] & (seq - 1))
            tokens.append(tok)
            grp = x_buf[tok >> 5, (tok >> 3) & 3].astype(_F32)
            one = jnp.sum(jnp.where(sub_d == (tok & 7), grp, 0.0), axis=0, keepdims=True)
            x_sel = jnp.where(sub_d == i, one, x_sel)
        order = picked >> (seq.bit_length() - 1)
        bits = jnp.where(order >= 0x8000, order - 0x8000, 0xFFFF - order)
        r_sel = jax.nn.sigmoid(pltpu.bitcast(bits << 16, _F32))

        for c in ffn_copies:
            c.wait()
        xb = x_sel.astype(_BF16)
        act = []
        for j in range(f_blk):
            gt = _dot(xb, _as_bf16(wg[j]))
            up = _dot(xb, _as_bf16(wu[j]))
            act.append(gt * jax.nn.sigmoid(gt) * up)
        act = jnp.concatenate(act, axis=1).astype(_BF16)
        y = [_dot(act, _as_bf16(wd[j])) * r_sel for j in range(n_blk)]
        for i, tok in enumerate(tokens):
            at = pl.ds(tok, 1)
            keep = 1.0 - g_buf[at, :]
            acc_buf[at, :] += jnp.concatenate([keep * yj[i:i + 1] for yj in y], axis=1)

    def weight(m, h, part):
        blocks = d_model // 32
        words = wqkv[m, h // 2, part * blocks:(part + 1) * blocks, h % 2]
        return _as_bf16(words.reshape(d_model // 4, _LANES))

    pad = jnp.zeros((8, _LANES), _F32)

    def segment(s, mem, prev):
        n_q, n_k = (32, 48) if prev is None else (48, 64)
        row, col = _iota((n_q, n_k), 0), _iota((n_q, n_k), 1)
        earlier = (row >= 32) & (row < 40)
        own = (earlier & (col >= 40) & (col < 56)) | (~earlier & (col < 40))
        last = jnp.where(row < 8, 39, jnp.where(row < 32, row + 8,
                                                jnp.where(row < 40, row + 16, row - 32)))
        visible = own & (col <= last)
        hidden = jnp.where(own, _MASKED, -jnp.inf).astype(_F32)

        xs = x_buf[s, 1:4].reshape(24, d_model).astype(_F32)
        full = jnp.concatenate([mem, xs], axis=0)
        h = [full[:, :d_model // 2].astype(_BF16), full[:, d_model // 2:].astype(_BF16)]

        def first(m, hd, seg, rows=8):
            return qkv0[m, hd, pl.ds(pl.multiple_of(seg * 8, 8), rows), :]

        q, k, v, e, o, keep, begun = {}, {}, {}, {}, {}, {}, {}

        def begin(hd):
            begun[hd] = [_dot(h[0], weight(m, hd, 0)) for m in range(3)]

        def project(hd):
            y = []
            for m in range(3):
                t = begun[hd][m] if hd in begun else _dot(h[0], weight(m, hd, 0))
                y.append(_dot(h[1], weight(m, hd, 1)) + t)
            keep[hd] = (y[1][:8], y[2][:8])
            if prev is not None:
                y[0] = jnp.concatenate([y[0], first(0, hd, s - 1, 16)], axis=0)
            q[hd] = y[0].astype(_BF16)
            for m, dst in ((1, k), (2, v)):
                rows = [y[m][:8], first(m, hd, s), y[m][8:]]
                if prev is not None:
                    rows += [prev[hd][m - 1], first(m, hd, s - 1)]
                dst[hd] = jnp.concatenate(rows + [pad], axis=0).astype(_BF16)

        def attend(hd):
            sc = lax.dot_general(q[hd], k[hd], _NT, preferred_element_type=_F32)
            sc = jnp.where(visible, sc * scale, hidden)
            ex = jnp.exp(sc - jnp.max(sc, axis=1, keepdims=True))
            tot = jnp.sum(ex, axis=1, keepdims=True)
            e[hd] = (ex * pltpu.reciprocal(tot, full_range=False)).astype(_BF16)

        def combine(hd):
            o[hd] = _dot(e[hd], v[hd]).astype(_BF16)

        def out_proj(h0, h1, j, acc):
            for hd in range(h0, h1):
                t = _dot(o[hd], _as_bf16(wo[j, hd * 64:(hd + 1) * 64, :]))
                acc = t if acc is None else t + acc
            return acc

        if prev is not None:
            for hd in range(SPLIT):
                begin(hd)
        for i in range(0, n_heads, 2):
            project(i)
            project(i + 1)
            for hd in (i - LAG_A, i + 1 - LAG_A):
                if hd >= 0:
                    attend(hd)
            for hd in (i - LAG_C, i + 1 - LAG_C):
                if hd >= 0:
                    combine(hd)
        half = n_heads // 2
        part = []
        for j in range(n_blk):
            part.append(out_proj(0, half, j, None))
            for kind, hd in TAIL.get(j, ()):
                (attend if kind == "a" else combine)(n_heads + hd)
        a = jnp.concatenate(
            [out_proj(half, n_heads, j, part[j]) for j in range(n_blk)], axis=1)
        return a, keep

    def emit(s, b, a):
        rows = pl.ds(pl.multiple_of(s * 32 + b * 8, 8), 8)
        t = acc_buf[rows, :] + jnp.tile(g_buf[rows, :], (1, n_blk)) * a
        acc_buf[rows, :] = t
        out_buf[s, b] = t.astype(out_buf.dtype)

    def two_segments(i, mem):
        @pl.when(i == _FFN_AT)
        def _():
            routed_ffn()
            for s in range(2 * _FFN_AT):
                for b in range(4):
                    out_buf[s, b] = acc_buf[s * 32 + b * 8:s * 32 + b * 8 + 8, :].astype(
                        out_buf.dtype)
            out_copy(0, 2 * _FFN_AT).start()

        @pl.when(i > _FFN_AT)
        def _():
            out_copy(2 * i - 2, 2).start()

        a, keep = segment(2 * i, mem, None)
        for b in range(1, 4):
            emit(2 * i, b, a[8 * b:8 * b + 8])
        a, _ = segment(2 * i + 1, a[:8], keep)
        for b in range(1, 4):
            emit(2 * i + 1, b, a[8 * b:8 * b + 8])
        emit(2 * i, 0, a[32:40])
        emit(2 * i + 1, 0, a[40:48])
        return a[:8]

    with jax.named_scope('S_steps'):
        lax.fori_loop(0, n_seg // 2, two_segments, mem0_ref[...].astype(_F32))
    out_copy(n_seg - 2, 2).start()
    out_copy(0, n_seg).wait()


@functools.partial(jax.jit, static_argnames=("A_seg_len",))
def pallas_gated_mix__memory_aug_recurrent_mem_tr__moe_arch_mod__prompt_kernel(
    A_x, A_mem0, A_Wq, A_Wk, A_Wv, A_Wo, A_seg_len,
    B_x, B_w_r, B_w_gate, B_w_up, B_w_down, gate_w,
):
    del B_x
    batch, seq, d_model = A_x.shape
    _, n_heads, d_head = A_Wq.shape
    d_ff = B_w_gate.shape[1]
    assert batch == 1 and A_seg_len == 32 and A_mem0.shape[1] == 8 and d_head == _LANES
    assert seq % 1024 == 0 and seq & (seq - 1) == 0 and d_model == 8 * _LANES
    n_seg = seq // A_seg_len
    n_blk, f_blk = d_model // _LANES, d_ff // _LANES

    def by_pair(w):
        return w.reshape(d_model // 16, 2, 8, n_heads, d_head)

    hbm = pl.BlockSpec(memory_space=pl.ANY)
    vmem = pl.BlockSpec(memory_space=pltpu.VMEM)
    out = pl.pallas_call(
        functools.partial(_kernel, n_seg=n_seg, n_heads=n_heads, d_model=d_model,
                          d_ff=d_ff, scale=d_head ** -0.5),
        out_shape=jax.ShapeDtypeStruct((n_seg, 4, 8, d_model), A_x.dtype),
        in_specs=[hbm, vmem, hbm, hbm, hbm, hbm, vmem, vmem, hbm, hbm, hbm],
        out_specs=hbm,
        scratch_shapes=[
            pltpu.VMEM((n_seg, 4, 8, d_model), A_x.dtype),
            pltpu.VMEM((n_seg * 4, d_model), _U32),
            pltpu.VMEM((3, n_heads // 2, d_model // 16, 2, 8, _LANES), _U32),
            pltpu.VMEM((n_blk, n_heads * d_head // 2, _LANES), _U32),
            pltpu.VMEM((f_blk, d_model // 2, _LANES), _U32),
            pltpu.VMEM((f_blk, d_model // 2, _LANES), _U32),
            pltpu.VMEM((n_blk, d_ff // 2, _LANES), _U32),
            pltpu.VMEM((3, n_heads, n_seg * 8, _LANES), _F32),
            pltpu.VMEM((seq, d_model), _F32),
            pltpu.VMEM((seq, _LANES), _F32),
            pltpu.VMEM((seq // (8 * _LANES), 8, _LANES), _F32),
            pltpu.VMEM((n_seg, 4, 8, d_model), A_x.dtype),
            pltpu.SemaphoreType.DMA((3, n_heads // 2)),
            pltpu.SemaphoreType.DMA((1,)),
            pltpu.SemaphoreType.DMA((n_heads // 2,)),
            pltpu.SemaphoreType.DMA((1,)),
            pltpu.SemaphoreType.DMA((1,)),
            pltpu.SemaphoreType.DMA((1,)),
        ],
        compiler_params=pltpu.CompilerParams(vmem_limit_bytes=120 * 2**20),
        name="gated_rmt_mod",
    )(
        A_x.reshape(n_seg, 4, 8, d_model),
        A_mem0.reshape(8, d_model),
        by_pair(A_Wq), by_pair(A_Wk), by_pair(A_Wv),
        A_Wo.reshape(n_heads * d_head, d_model),
        B_w_r.reshape(n_blk, _LANES), gate_w.reshape(n_blk, _LANES),
        B_w_gate, B_w_up, B_w_down,
    )
    return out.reshape(batch, seq, d_model)
```

```python
import functools

import jax
import jax.numpy as jnp
from jax import lax
import jax.experimental.pallas as pl
import jax.experimental.pallas.tpu as pltpu

_LANES = 128
_TOP_C = 8
_MASKED = -1000000000.0
_KEY_BASE = 0x20000000
_FFN_AT = 2
LAG_A, LAG_C = 2, 4
TAIL = {1:(('a',-2),('a',-1)),3:(('c',-4),('c',-3)),6:(('c',-2),('c',-1))}
SPLIT = 2
UNROLL = 2
AHEAD = 0
FFN_EARLY = 0
STRASSEN = False
NOCHK = False
WO_PER = 1
XAT = 1
FLAGS = {'XLA_TPU_EVENLY_DISTRIBUTE_CRITICAL_NODES': True}

_BF16 = jnp.bfloat16
_F32 = jnp.float32
_U32 = jnp.uint32
_NT = (((1,), (1,)), ((), ()))


def _as_bf16(words):
    return pltpu.bitcast(words, _BF16)


def _as_words(rows):
    return pltpu.bitcast(rows, _U32)


def _dot(a, b):
    return jnp.dot(a, b, preferred_element_type=_F32)


def _iota(shape, dim):
    return lax.broadcasted_iota(jnp.int32, shape, dim)


def _kernel(x_hbm, mem0_hbm, wq_hbm, wk_hbm, wv_hbm, wo_hbm, wr_hbm, gw_hbm,
            wg_hbm, wu_hbm, wd_hbm, out_hbm,
            x_buf, x0_buf, wqkv, wo, wg, wu, wd, qkv0, acc_buf, g_buf, r_buf, out_buf,
            mem0_ref, wr_ref, gw_ref, w_sem, x0_sem, x_sem, wo_sem, ffn_sem, out_sem, small_sem,
            *, n_seg, n_heads, d_model, d_ff, scale):
    n_pairs = n_heads // 2
    n_blk = d_model // _LANES
    f_blk = d_ff // _LANES
    n_rows0 = n_seg * 8
    seq = n_seg * 32
    span = n_seg // n_pairs

    def w_copy(m, p):
        src = (wq_hbm, wk_hbm, wv_hbm)[m].bitcast(_U32)
        return pltpu.make_async_copy(src.at[:, :, :, p, :], wqkv.at[m, p], w_sem.at[m, p])

    def col_copy(hbm, dst, j, sem):
        cols = pl.ds(j * _LANES if isinstance(j, int) else pl.multiple_of(j * _LANES, _LANES), _LANES)
        return pltpu.make_async_copy(hbm.bitcast(_U32).at[:, cols], dst.at[j], sem)

    def x_copy(p):
        src = x_hbm.at[pl.ds(p * span, span), pl.ds(1, 3)]
        return pltpu.make_async_copy(src, x_buf.at[pl.ds(p * span, span), pl.ds(1, 3)], x_sem.at[p])

    def out_copy(first, count):
        at = pl.ds(first, count)
        return pltpu.make_async_copy(out_buf.at[at], out_hbm.at[at], out_sem.at[0])

    x0_copy = pltpu.make_async_copy(
        x_hbm.at[:, pl.ds(0, 1)], x_buf.at[pl.ds(0, n_seg), pl.ds(0, 1)], x0_sem.at[0])
    ffn_copies = ([col_copy(wg_hbm, wg, j, ffn_sem.at[0]) for j in range(f_blk)]
                  + [col_copy(wu_hbm, wu, j, ffn_sem.at[0]) for j in range(f_blk)]
                  + [col_copy(wd_hbm, wd, j, ffn_sem.at[0]) for j in range(n_blk)])

    lane = _iota((8, _LANES), 1)
    n_keys = seq // (8 * _LANES)

    def row_dot(xs, w):
        t = xs[:, :_LANES] * w[0:1]
        for j in range(1, n_blk):
            t = t + xs[:, j * _LANES:(j + 1) * _LANES] * w[j:j + 1]
        return jnp.sum(t, axis=1, keepdims=True)

    def fetch(p):
        for m in range(3):
            w_copy(m, p).start()
        x_copy(p).start()

    def route(s, scores):
        xs = x_buf[s].reshape(32, d_model).astype(_F32)
        z = row_dot(xs, gw_ref[...].astype(_F32))
        g = jax.nn.sigmoid(z)
        r = row_dot(xs, wr_ref[...].astype(_F32))
        rows = pl.ds(pl.multiple_of(s * 32, 32), 32)
        g_buf[rows, :] = jnp.broadcast_to(g, (32, _LANES))
        acc_buf[rows, :] = (1.0 - g) * xs
        scores = list(scores)
        for b in range(4):
            for u in range(n_keys):
                scores[u] = jnp.where(
                    lane == 4 * s + b - u * _LANES, r[8 * b:8 * b + 8], scores[u])
        return tuple(scores)

    hr, hd_ = n_rows0 // 2, d_model // 2

    def project_first(m, p, between):
        raw = wqkv[m, p].reshape(d_model, _LANES)
        even = pltpu.bitcast(raw << 16, _F32)
        odd = pltpu.bitcast(raw & jnp.uint32(0xFFFF0000), _F32)
        if not STRASSEN:
            x0 = _as_bf16(x0_buf[...])
            for par, half in enumerate((even, odd)):
                w = half.astype(_BF16)
                wqkv[m, p, :, par] = _as_words(w).reshape(d_model // 16, 8, _LANES)
                qkv0[m, 2 * p + par] = _dot(x0, w)
                between()
            return
        b11, b21, b12, b22 = even[:hd_], even[hd_:], odd[:hd_], odd[hd_:]

        def prod(i, b):
            return _dot(_as_bf16(x0_buf[i]), b.astype(_BF16))

        m1 = prod(0, b11 + b22)
        u = prod(6, b21 + b22) + m1
        w = prod(5, b11 + b12) + m1
        between()
        m5 = prod(4, b22)
        m4 = prod(3, b21 - b11)
        qkv0[m, 2 * p, :hr] = u + m4 - m5
        m2 = prod(1, b11)
        qkv0[m, 2 * p, hr:] = m2 + m4
        between()
        for par, half in enumerate((even, odd)):
            wqkv[m, p, :, par] = _as_words(half.astype(_BF16)).reshape(d_model // 16, 8, _LANES)
        m3 = prod(2, b12 - b22)
        qkv0[m, 2 * p + 1, :hr] = m3 + m5
        qkv0[m, 2 * p + 1, hr:] = w - m2 + m3

    def wo_copy(i):
        rows = n_heads * _LANES // 4
        at = pl.ds((i % 2) * rows, rows)
        j = i // 2
        cols = pl.ds(j * _LANES if isinstance(j, int) else pl.multiple_of(j * _LANES, _LANES), _LANES)
        return pltpu.make_async_copy(wo_hbm.bitcast(_U32).at[at, cols], wo.at[j, at], wo_sem.at[0])

    small = [pltpu.make_async_copy(src, dst, small_sem.at[0])
             for src, dst in ((wr_hbm, wr_ref), (gw_hbm, gw_ref), (mem0_hbm, mem0_ref))]
    x0_copy.start()
    w_copy(0, 0).start()
    for c in small:
        c.start()
    x0_copy.wait()
    w_copy(1, 0).start()
    w_copy(2, 0).start()
    if STRASSEN:
        xa = x_buf[:n_seg, 0].reshape(n_rows0, d_model).astype(_F32)
        a11, a12, a21, a22 = xa[:hr, :hd_], xa[:hr, hd_:], xa[hr:, :hd_], xa[hr:, hd_:]
        for i, a in enumerate((a11 + a22, a21 + a22, a11, a22, a11 + a12, a21 - a11, a12 - a22)):
            x0_buf[i] = _as_words(a.astype(_BF16))
    else:
        x0_buf[...] = _as_words(x_buf[:n_seg, 0].reshape(n_rows0, d_model))
    w_copy(0, 0).wait()
    x_copy(0).start()
    project_first(0, 0, lambda: None)
    fetch(1)
    for c in small:
        c.wait()
    w_copy(1, 0).wait()
    w_copy(2, 0).wait()
    x_copy(0).wait()

    def pair(p, mats, scores):
        state = [scores]
        todo = [p * span + t for t in range(span)]

        def between():
            if todo:
                state[0] = route(todo.pop(0), state[0])

        between()
        for m in mats:
            project_first(m, p, between)
        assert not todo
        return state[0]

    scores = pair(0, (1, 2), tuple(jnp.zeros((8, _LANES), _F32) for _ in range(n_keys)))
    fetch(2)
    wo_copy(0).start()
    wo_copy(1).start()

    def prologue(p, scores):
        for m in range(3):
            w_copy(m, p).wait()
        x_copy(p).wait()
        scores = pair(p, (0, 1, 2), scores)

        @pl.when(p + 2 < n_pairs)
        def _():
            fetch(p + 2)
            wo_copy(p + 1).start()

        @pl.when(p + 2 == n_pairs)
        def _():
            wo_copy(n_pairs - 1).start()
            for c in ffn_copies[:FFN_EARLY]:
                c.start()

        return scores

    with jax.named_scope('S_prologue'):
        scores = lax.fori_loop(1, n_pairs, prologue, scores)
    for u in range(n_keys):
        r_buf[u] = scores[u]

    for c in ffn_copies[FFN_EARLY:]:
        c.start()
    for i in range(n_pairs):
        wo_copy(i).wait()

    def routed_ffn():
        sub = _iota((8, _LANES), 0)
        keys = []
        for u in range(n_keys):
            r = r_buf[u].astype(_BF16).astype(_F32)
            bits = lax.shift_right_logical(
                pltpu.bitcast(jnp.where(r == 0.0, 0.0, r), jnp.int32), 16)
            order = jnp.where(bits >= 0x8000, 0xFFFF - bits, bits + 0x8000)
            order = jnp.where(r != r, 0, order)
            token = (lane + u * _LANES) * 8 + sub
            keys.append(pltpu.bitcast(_KEY_BASE + order * seq + (seq - 1 - token), _F32))

        sub_d = _iota((8, d_model), 0)
        picked = jnp.zeros((8, _LANES), jnp.int32)
        x_sel = jnp.zeros((8, d_model), _F32)
        tokens = []
        for i in range(_TOP_C):
            best = functools.reduce(jnp.maximum, keys)
            best = jnp.max(jnp.max(best, axis=1, keepdims=True), axis=0, keepdims=True)
            keys = [jnp.where(kk == best, 0.0, kk) for kk in keys]
            code = pltpu.bitcast(jnp.broadcast_to(best, (8, _LANES)), jnp.int32) - _KEY_BASE
            picked = jnp.where(sub == i, code, picked)
            tok = seq - 1 - (code[0, 0] & (seq - 1))
            tokens.append(tok)
            grp = x_buf[tok >> 5, (tok >> 3) & 3].astype(_F32)
            one = jnp.sum(jnp.where(sub_d == (tok & 7), grp, 0.0), axis=0, keepdims=True)
            x_sel = jnp.where(sub_d == i, one, x_sel)
        order = picked >> (seq.bit_length() - 1)
        bits = jnp.where(order >= 0x8000, order - 0x8000, 0xFFFF - order)
        r_sel = jax.nn.sigmoid(pltpu.bitcast(bits << 16, _F32))

        for c in ffn_copies:
            c.wait()
        xb = x_sel.astype(_BF16)
        act = []
        for j in range(f_blk):
            gt = _dot(xb, _as_bf16(wg[j]))
            up = _dot(xb, _as_bf16(wu[j]))
            act.append(gt * jax.nn.sigmoid(gt) * up)
        act = jnp.concatenate(act, axis=1).astype(_BF16)
        y = [_dot(act, _as_bf16(wd[j])) * r_sel for j in range(n_blk)]
        for i, tok in enumerate(tokens):
            at = pl.ds(tok, 1)
            keep = 1.0 - g_buf[at, :]
            acc_buf[at, :] += jnp.concatenate([keep * yj[i:i + 1] for yj in y], axis=1)

    def weight(m, h, part):
        blocks = d_model // 32
        words = wqkv[m, h // 2, part * blocks:(part + 1) * blocks, h % 2]
        return _as_bf16(words.reshape(d_model // 4, _LANES))

    pad = jnp.zeros((8, _LANES), _F32)

    def segment(s, mem, prev, split):
        n_q, n_k = (32, 48) if prev is None else (48, 64)
        row, col = _iota((n_q, n_k), 0), _iota((n_q, n_k), 1)
        earlier = (row >= 32) & (row < 40)
        own = (earlier & (col >= 40) & (col < 56)) | (~earlier & (col < 40))
        last = jnp.where(row < 8, 39, jnp.where(row < 32, row + 8,
                                                jnp.where(row < 40, row + 16, row - 32)))
        visible = own & (col <= last)
        hidden = jnp.where(own, _MASKED, -jnp.inf).astype(_F32)

        xs = x_buf[s, 1:4].reshape(24, d_model).astype(_F32)
        full = jnp.concatenate([mem, xs], axis=0)
        h = [full[:, :d_model // 2].astype(_BF16), full[:, d_model // 2:].astype(_BF16)]

        def first(m, hd, seg, rows=8):
            return qkv0[m, hd, pl.ds(pl.multiple_of(seg * 8, 8), rows), :]

        q, k, v, e, o, keep, begun = {}, {}, {}, {}, {}, {}, {}

        def begin(hd):
            begun[hd] = [_dot(h[0], weight(m, hd, 0)) for m in range(3)]

        def project(hd):
            y = []
            for m in range(3):
                t = begun[hd][m] if hd in begun else _dot(h[0], weight(m, hd, 0))
                y.append(_dot(h[1], weight(m, hd, 1)) + t)
            keep[hd] = (y[1][:8], y[2][:8])
            if prev is not None:
                y[0] = jnp.concatenate([y[0], first(0, hd, s - 1, 16)], axis=0)
            q[hd] = y[0].astype(_BF16)
            for m, dst in ((1, k), (2, v)):
                rows = [y[m][:8], first(m, hd, s), y[m][8:]]
                if prev is not None:
                    rows += [prev[hd][m - 1], first(m, hd, s - 1)]
                dst[hd] = jnp.concatenate(rows + [pad], axis=0).astype(_BF16)

        def attend(hd):
            sc = lax.dot_general(q[hd], k[hd], _NT, preferred_element_type=_F32)
            sc = jnp.where(visible, sc * scale, hidden)
            ex = jnp.exp(sc - jnp.max(sc, axis=1, keepdims=True))
            tot = jnp.sum(ex, axis=1, keepdims=True)
            e[hd] = (ex * pltpu.reciprocal(tot, full_range=False)).astype(_BF16)

        def combine(hd):
            o[hd] = _dot(e[hd], v[hd]).astype(_BF16)

        def out_proj(h0, h1, j, acc):
            for hd in range(h0, h1):
                t = _dot(o[hd], _as_bf16(wo[j, hd * 64:(hd + 1) * 64, :]))
                acc = t if acc is None else t + acc
            return acc

        for hd in range(split):
            begin(hd)
        for i in range(0, n_heads, 2):
            project(i)
            project(i + 1)
            for hd in (i - LAG_A, i + 1 - LAG_A):
                if hd >= 0:
                    attend(hd)
            for hd in (i - LAG_C, i + 1 - LAG_C):
                if hd >= 0:
                    combine(hd)
        half = n_heads // 2
        part = []
        for j in range(n_blk):
            part.append(out_proj(0, half, j, None))
            for kind, hd in TAIL.get(j, ()):
                (attend if kind == "a" else combine)(n_heads + hd)
        a = jnp.concatenate(
            [out_proj(half, n_heads, j, part[j]) for j in range(n_blk)], axis=1)
        return a, keep

    def emit(s, b, a):
        rows = pl.ds(pl.multiple_of(s * 32 + b * 8, 8), 8)
        t = acc_buf[rows, :] + jnp.tile(g_buf[rows, :], (1, n_blk)) * a
        acc_buf[rows, :] = t
        out_buf[s, b] = t.astype(out_buf.dtype)

    batch = 2 * UNROLL

    def segments(i, mem):
        @pl.when(i == _FFN_AT)
        def _():
            routed_ffn()
            for s in range(batch * _FFN_AT):
                for b in range(4):
                    out_buf[s, b] = acc_buf[s * 32 + b * 8:s * 32 + b * 8 + 8, :].astype(
                        out_buf.dtype)
            out_copy(0, batch * _FFN_AT).start()

        @pl.when(i > _FFN_AT)
        def _():
            out_copy(batch * (i - 1), batch).start()

        for u in range(UNROLL):
            s = batch * i + 2 * u
            a, keep = segment(s, mem, None, SPLIT if u else 0)
            for b in range(1, 4):
                emit(s, b, a[8 * b:8 * b + 8])
            a, _ = segment(s + 1, a[:8], keep, SPLIT)
            for b in range(1, 4):
                emit(s + 1, b, a[8 * b:8 * b + 8])
            emit(s, 0, a[32:40])
            emit(s + 1, 0, a[40:48])
            mem = a[:8]
        return mem

    with jax.named_scope('S_steps'):
        lax.fori_loop(0, n_seg // batch, segments, mem0_ref[...].astype(_F32))
    out_copy(n_seg - batch, batch).start()
    out_copy(0, n_seg).wait()


@functools.partial(jax.jit, static_argnames=("A_seg_len",))
def pallas_gated_mix__memory_aug_recurrent_mem_tr__moe_arch_mod__prompt_kernel(
    A_x, A_mem0, A_Wq, A_Wk, A_Wv, A_Wo, A_seg_len,
    B_x, B_w_r, B_w_gate, B_w_up, B_w_down, gate_w,
):
    del B_x
    batch, seq, d_model = A_x.shape
    _, n_heads, d_head = A_Wq.shape
    d_ff = B_w_gate.shape[1]
    assert batch == 1 and A_seg_len == 32 and A_mem0.shape[1] == 8 and d_head == _LANES
    assert seq % 1024 == 0 and seq & (seq - 1) == 0 and d_model == 8 * _LANES
    n_seg = seq // A_seg_len
    n_blk, f_blk = d_model // _LANES, d_ff // _LANES

    def by_pair(w):
        return w.reshape(d_model // 16, 2, 8, n_heads, d_head)

    hbm = pl.BlockSpec(memory_space=pl.ANY)
    vmem = pl.BlockSpec(memory_space=pltpu.VMEM)
    out = pl.pallas_call(
        functools.partial(_kernel, n_seg=n_seg, n_heads=n_heads, d_model=d_model,
                          d_ff=d_ff, scale=d_head ** -0.5),
        out_shape=jax.ShapeDtypeStruct((n_seg, 4, 8, d_model), A_x.dtype),
        in_specs=[hbm] * 11,
        out_specs=hbm,
        scratch_shapes=[
            pltpu.VMEM((n_seg + AHEAD * 4, 4, 8, d_model), A_x.dtype),
            pltpu.VMEM((7, n_seg * 2, d_model // 2) if STRASSEN else (n_seg * 4, d_model), _U32),
            pltpu.VMEM((3, n_heads // 2 + AHEAD, d_model // 16, 2, 8, _LANES), _U32),
            pltpu.VMEM((n_blk, n_heads * d_head // 2, _LANES), _U32),
            pltpu.VMEM((f_blk, d_model // 2, _LANES), _U32),
            pltpu.VMEM((f_blk, d_model // 2, _LANES), _U32),
            pltpu.VMEM((n_blk, d_ff // 2, _LANES), _U32),
            pltpu.VMEM((3, n_heads, n_seg * 8, _LANES), _F32),
            pltpu.VMEM((seq, d_model), _F32),
            pltpu.VMEM((seq, _LANES), _F32),
            pltpu.VMEM((seq // (8 * _LANES), 8, _LANES), _F32),
            pltpu.VMEM((n_seg, 4, 8, d_model), A_x.dtype),
            pltpu.VMEM((8, d_model), A_mem0.dtype),
            pltpu.VMEM((n_blk, _LANES), B_w_r.dtype),
            pltpu.VMEM((n_blk, _LANES), gate_w.dtype),
            pltpu.SemaphoreType.DMA((3, n_heads // 2 + AHEAD)),
            pltpu.SemaphoreType.DMA((1,)),
            pltpu.SemaphoreType.DMA((n_heads // 2 + AHEAD,)),
            pltpu.SemaphoreType.DMA((1,)),
            pltpu.SemaphoreType.DMA((1,)),
            pltpu.SemaphoreType.DMA((1,)),
            pltpu.SemaphoreType.DMA((1,)),
        ],
        compiler_params=pltpu.CompilerParams(vmem_limit_bytes=120 * 2**20, flags=FLAGS, disable_bounds_checks=NOCHK),
        name="gated_rmt_mod",
    )(
        A_x.reshape(n_seg, 4, 8, d_model),
        A_mem0.reshape(8, d_model),
        by_pair(A_Wq), by_pair(A_Wk), by_pair(A_Wv),
        A_Wo.reshape(n_heads * d_head, d_model),
        B_w_r.reshape(n_blk, _LANES), gate_w.reshape(n_blk, _LANES),
        B_w_gate, B_w_up, B_w_down,
    )
    return out.reshape(batch, seq, d_model)
```

```python
import functools

import jax
import jax.numpy as jnp
from jax import lax
import jax.experimental.pallas as pl
import jax.experimental.pallas.tpu as pltpu

_LANES = 128
_TOP_C = 8
_MASKED = -1000000000.0
_KEY_BASE = 0x20000000
LAG_A, LAG_C = 2, 4
TAIL = {1: (('a', -2), ('a', -1)), 3: (('c', -4), ('c', -3)), 6: (('c', -2), ('c', -1))}
SPLIT = 2
FFN_SKIP = 4
FLAGS = {'XLA_TPU_EVENLY_DISTRIBUTE_CRITICAL_NODES': True}

_BF16 = jnp.bfloat16
_F32 = jnp.float32
_U32 = jnp.uint32
_NT = (((1,), (1,)), ((), ()))


def _as_bf16(words):
    return pltpu.bitcast(words, _BF16)


def _as_words(rows):
    return pltpu.bitcast(rows, _U32)


def _dot(a, b, acc=None):
    y = jnp.dot(a, b, preferred_element_type=_F32)
    return y if acc is None else y + acc


def _iota(shape, dim):
    return lax.broadcasted_iota(jnp.int32, shape, dim)


def _left_factor(i, a):
    return (lambda: a(0, 0) + a(1, 1), lambda: a(1, 0) + a(1, 1), lambda: a(0, 0),
            lambda: a(1, 1), lambda: a(0, 0) + a(0, 1), lambda: a(1, 0) - a(0, 0),
            lambda: a(0, 1) - a(1, 1))[i]()


def _strassen(prod, plain, b, put, between):
    m5 = prod(4, lambda *k: plain(1, *k), None)
    m3 = prod(2, lambda *k: b(0, 1, *k) - b(1, 1, *k), None)
    put(0, 1, m3 + m5)
    m2 = prod(1, lambda *k: plain(0, *k), None)
    w = m3 - m2
    between()
    m4 = prod(3, lambda *k: b(1, 0, *k) - b(0, 0, *k), None)
    put(1, 0, m2 + m4)
    u = m4 - m5
    m1 = prod(0, lambda *k: b(0, 0, *k) + b(1, 1, *k), None)
    between()
    put(0, 0, prod(6, lambda *k: b(1, 0, *k) + b(1, 1, *k), u + m1))
    put(1, 1, prod(5, lambda *k: b(0, 0, *k) + b(0, 1, *k), w + m1))


def _kernel(x_hbm, mem0_hbm, wq_hbm, wk_hbm, wv_hbm, wo_hbm, wr_hbm, gw_hbm,
            wg_hbm, wu_hbm, wd_hbm, out_hbm,
            x_buf, x0_buf, stage, wqkv, wo, wg, wu, wd, qkv0, o0_buf, acc_buf, g_buf, out_buf,
            mem0_buf, wr_buf, gw_buf, tok_buf,
            w_sem, x_sem, x0_sem, wo_sem, ffn_sem, small_sem, out_sem,
            *, n_seg, n_heads, d_model, d_ff, scale):
    n_pairs = n_heads // 2
    n_blk = d_model // _LANES
    f_blk = d_ff // _LANES
    seq = n_seg * 32
    span = n_seg // n_pairs
    half_rows, half_d = n_seg * 4, d_model // 2

    def w_copy(m, p):
        src = (wq_hbm, wk_hbm, wv_hbm)[m].bitcast(_U32)
        return pltpu.make_async_copy(src.at[:, p, :], stage.at[p % 2, m], w_sem.at[p % 2, m])

    def x_copy(p):
        at = (pl.ds(p * span, span), pl.ds(1, 3))
        return pltpu.make_async_copy(x_hbm.at[at], x_buf.at[at], x_sem.at[p % 2])

    def wo_copy(i):
        rows = n_heads * _LANES // 4
        at, j = pl.ds((i % 2) * rows, rows), i // 2
        cols = pl.ds(pl.multiple_of(j * _LANES, _LANES), _LANES)
        return pltpu.make_async_copy(
            wo_hbm.bitcast(_U32).at[at, cols], wo.at[j, at], wo_sem.at[0])

    def col_copy(hbm, dst, j):
        src = hbm.bitcast(_U32).at[:, pl.ds(j * _LANES, _LANES)]
        return pltpu.make_async_copy(src, dst.at[j], ffn_sem.at[0])

    def out_copy(at, sem):
        return pltpu.make_async_copy(out_buf.at[at], out_hbm.at[at], out_sem.at[sem])

    x0_copy = pltpu.make_async_copy(
        x_hbm.at[:, pl.ds(0, 1)], x_buf.at[:, pl.ds(0, 1)], x0_sem.at[0])
    small_copies = [pltpu.make_async_copy(src, dst, small_sem.at[0])
                    for src, dst in ((wr_hbm, wr_buf), (gw_hbm, gw_buf), (mem0_hbm, mem0_buf))]
    ffn_copies = ([col_copy(wg_hbm, wg, j) for j in range(f_blk)]
                  + [col_copy(wu_hbm, wu, j) for j in range(f_blk)]
                  + [col_copy(wd_hbm, wd, j) for j in range(n_blk)])

    lane = _iota((8, _LANES), 1)
    n_keys = seq // (8 * _LANES)

    def row_dot(xs, w_buf):
        w = w_buf[...].astype(_F32)
        t = xs[:, :_LANES] * w[0:1]
        for j in range(1, n_blk):
            t = t + xs[:, j * _LANES:(j + 1) * _LANES] * w[j:j + 1]
        return jnp.sum(t, axis=1, keepdims=True)

    def route(s, scores):
        xs = x_buf[s].reshape(32, d_model).astype(_F32)
        g = jax.nn.sigmoid(row_dot(xs, gw_buf))
        r = row_dot(xs, wr_buf)
        rows = pl.ds(pl.multiple_of(s * 32, 32), 32)
        g_buf[rows, :] = jnp.broadcast_to(g, (32, _LANES))
        acc_buf[rows, :] = (1.0 - g) * xs
        scores = list(scores)
        for b in range(4):
            for u in range(n_keys):
                scores[u] = jnp.where(
                    lane == 4 * s + b - u * _LANES, r[8 * b:8 * b + 8], scores[u])
        return tuple(scores)

    def project_first(m, p, between=lambda: None, left=lambda i: x0_buf[i]):
        def plain(r):
            a, b = (stage[p % 2, m, pl.ds(r * half_d + t, half_d // 2, stride=2), :]
                    for t in range(2))
            words = ((a & jnp.uint32(0xFFFF)) | (b << 16),
                     (a >> 16) | (b & jnp.uint32(0xFFFF0000)))
            for c in range(2):
                wqkv[m, 2 * p + c, r * half_d // 2:(r + 1) * half_d // 2] = words[c]
            return _as_bf16(words[r])

        def block(r, c):
            words = stage[p % 2, m, r * half_d:(r + 1) * half_d]
            return pltpu.bitcast(words & jnp.uint32(0xFFFF0000) if c else words << 16, _F32)

        def prod(i, right, acc):
            return _dot(_as_bf16(left(i)), right().astype(_BF16), acc)

        def put(r, c, val):
            qkv0[m, 2 * p + c, r * half_rows:(r + 1) * half_rows] = val

        _strassen(prod, plain, block, put, between)

    def first_left(i):
        def a(r, c):
            rows = x_buf[r * n_seg // 2:(r + 1) * n_seg // 2, 0, :, c * half_d:(c + 1) * half_d]
            return rows.reshape(half_rows, half_d).astype(_F32)
        words = _as_words(_left_factor(i, a).astype(_BF16))
        x0_buf[i] = words
        return words

    def project_pair(p, mats, scores):
        state = [scores]
        todo = [p * span + t for t in range(span)]

        def between():
            if todo:
                state[0] = route(todo.pop(0), state[0])

        while len(todo) > 2 * len(mats):
            between()
        between()
        for m in mats:
            project_first(m, p, between)
        return state[0]

    def fetch(p):
        for m in range(3):
            w_copy(m, p).start()
        x_copy(p).start()

    x0_copy.start()
    w_copy(0, 0).start()
    x0_copy.wait()
    w_copy(1, 0).start()
    w_copy(2, 0).start()
    x_copy(0).start()
    for c in small_copies:
        c.start()
    w_copy(0, 0).wait()
    project_first(0, 0, left=first_left)
    for m in range(3):
        w_copy(m, 1).start()
    w_copy(1, 0).wait()
    project_first(1, 0)
    x_copy(1).start()
    w_copy(2, 0).wait()
    x_copy(0).wait()
    for c in small_copies:
        c.wait()
    scores = project_pair(0, (2,), tuple(jnp.zeros((8, _LANES), _F32) for _ in range(n_keys)))
    fetch(2)
    wo_copy(0).start()
    wo_copy(1).start()

    def prologue(p, scores):
        for m in range(3):
            w_copy(m, p).wait()
        x_copy(p).wait()
        scores = project_pair(p, (0, 1, 2), scores)

        @pl.when(p + 2 < n_pairs)
        def _():
            fetch(p + 2)

        @pl.when(p + 1 < n_pairs)
        def _():
            wo_copy(p + 1).start()

        return scores

    with jax.named_scope('S_prologue'):
        scores = lax.fori_loop(1, n_pairs, prologue, scores)
    for c in ffn_copies:
        c.start()
    for i in range(n_pairs):
        wo_copy(i).wait()

    def weight(m, h, part):
        return _as_bf16(wqkv[m, h, part * half_d // 2:(part + 1) * half_d // 2])

    pad = jnp.zeros((8, _LANES), _F32)

    def segment(s, mem, prev, split, early=None):
        n_q, n_k = (32, 48) if prev is None else (48, 64)
        row, col = _iota((n_q, n_k), 0), _iota((n_q, n_k), 1)
        earlier = (row >= 32) & (row < 40)
        own = (earlier & (col >= 40) & (col < 56)) | (~earlier & (col < 40))
        last = jnp.where(row < 8, 39, jnp.where(row < 32, row + 8,
                                                jnp.where(row < 40, row + 16, row - 32)))
        visible = own & (col <= last)
        hidden = jnp.where(own, _MASKED, -jnp.inf).astype(_F32)

        xs = x_buf[s, 1:4].reshape(24, d_model).astype(_F32)
        full = jnp.concatenate([mem, xs], axis=0)
        h = [full[:, :half_d].astype(_BF16), full[:, half_d:].astype(_BF16)]

        def first(m, hd, seg, rows=8):
            return qkv0[m, hd, pl.ds(pl.multiple_of(seg * 8, 8), rows), :]

        q, k, v, e, o, o0, keep, begun = {}, {}, {}, {}, {}, {}, {}, {}

        def begin(hd):
            begun[hd] = [_dot(h[0], weight(m, hd, 0)) for m in range(3)]

        def project(hd):
            y = []
            for m in range(3):
                t = begun[hd][m] if hd in begun else _dot(h[0], weight(m, hd, 0))
                y.append(_dot(h[1], weight(m, hd, 1), t))
            keep[hd] = (y[1][:8], y[2][:8])
            if prev is not None:
                y[0] = jnp.concatenate([y[0], first(0, hd, s - 1, 16)], axis=0)
            q[hd] = y[0].astype(_BF16)
            for m, dst in ((1, k), (2, v)):
                rows = [y[m][:8], first(m, hd, s), y[m][8:]]
                if prev is not None:
                    rows += [prev[hd][m - 1], first(m, hd, s - 1)]
                dst[hd] = jnp.concatenate(rows + [pad], axis=0).astype(_BF16)

        def attend(hd):
            sc = lax.dot_general(q[hd], k[hd], _NT, preferred_element_type=_F32)
            sc = jnp.where(visible, sc * scale, hidden)
            ex = jnp.exp(sc - jnp.max(sc, axis=1, keepdims=True))
            tot = jnp.sum(ex, axis=1, keepdims=True)
            e[hd] = (ex * pltpu.reciprocal(tot, full_range=False)).astype(_BF16)

        def combine(hd):
            y = _dot(e[hd], v[hd])
            o[hd] = y[:32].astype(_BF16)
            if prev is not None:
                o0[hd] = y[32:]
                if early is not None and hd % 2:
                    early(hd // 2, o0)

        def out_proj(h0, h1, j, acc):
            for hd in range(h0, h1):
                acc = _dot(o[hd], _as_bf16(wo[j, hd * 64:(hd + 1) * 64, :]), acc)
            return acc

        for hd in range(split):
            begin(hd)
        for i in range(0, n_heads, 2):
            project(i)
            project(i + 1)
            for hd in (i - LAG_A, i + 1 - LAG_A):
                if hd >= 0:
                    attend(hd)
            for hd in (i - LAG_C, i + 1 - LAG_C):
                if hd >= 0:
                    combine(hd)
        half = n_heads // 2
        part = []
        for j in range(n_blk):
            part.append(out_proj(0, half, j, None))
            for kind, hd in TAIL.get(j, ()):
                (attend if kind == "a" else combine)(n_heads + hd)
        a = jnp.concatenate(
            [out_proj(half, n_heads, j, part[j]) for j in range(n_blk)], axis=1)
        for b in range(1, 4):
            rows = pl.ds(pl.multiple_of(s * 32 + b * 8, 8), 8)
            t = acc_buf[rows, :] + jnp.tile(g_buf[rows, :], (1, n_blk)) * a[8 * b:8 * b + 8]
            acc_buf[rows, :] = t
            out_buf[s, b] = t.astype(out_buf.dtype)
        return a[:8], (keep if prev is None else o0)

    sub, sub_d = _iota((8, _LANES), 0), _iota((8, d_model), 0)
    keys = []
    for u in range(n_keys):
        r = scores[u].astype(_BF16).astype(_F32)
        bits = lax.shift_right_logical(
            pltpu.bitcast(jnp.where(r == 0.0, 0.0, r), jnp.int32), 16)
        order = jnp.where(bits >= 0x8000, 0xFFFF - bits, bits + 0x8000)
        order = jnp.where(r != r, 0, order)
        token = (lane + u * _LANES) * 8 + sub
        keys.append(pltpu.bitcast(_KEY_BASE + order * seq + (seq - 1 - token), _F32))

    def pick(i, keys, picked, x_sel):
        best = functools.reduce(jnp.maximum, keys)
        best = jnp.max(jnp.max(best, axis=1, keepdims=True), axis=0, keepdims=True)
        keys = tuple(jnp.where(kk == best, 0.0, kk) for kk in keys)
        code = pltpu.bitcast(jnp.broadcast_to(best, (8, _LANES)), jnp.int32) - _KEY_BASE
        tok = seq - 1 - (code[0, 0] & (seq - 1))
        tok_buf[i] = tok
        grp = x_buf[tok >> 5, (tok >> 3) & 3].astype(_F32)
        one = jnp.sum(jnp.where(sub_d == (tok & 7), grp, 0.0), axis=0, keepdims=True)
        return keys, jnp.where(sub == i, code, picked), jnp.where(sub_d == i, one, x_sel)

    def four_segments(i, carry):
        mem, routing = carry
        s = 4 * i
        routing = pick(i, *routing)
        mem, keep = segment(s, mem, None, 0)
        mem, o_a = segment(s + 1, mem, keep, SPLIT)
        mem, keep = segment(s + 2, mem, None, SPLIT)

        def early(p, o_b):
            def a(r, c):
                return jnp.concatenate(
                    [t[2 * p + c][8 * r:8 * r + 8] for t in (o_a, o_b)], axis=0)
            for f in range(7):
                o0_buf[f, p, pl.ds(pl.multiple_of(i * 8, 8), 8), :] = _as_words(
                    _left_factor(f, a).astype(_BF16))

        mem, _ = segment(s + 3, mem, keep, SPLIT, early)
        out_copy((pl.ds(s, 4), pl.ds(1, 3)), 0).start()
        return mem, routing

    routing = (tuple(keys), jnp.zeros((8, _LANES), jnp.int32), jnp.zeros((8, d_model), _F32))
    with jax.named_scope('S_steps'):
        _, (_, picked, x_sel) = lax.fori_loop(
            0, n_seg // 4, four_segments, (mem0_buf[...].astype(_F32), routing))
    for c in ffn_copies:
        c.wait()

    n_fin = n_blk // 2
    f_per = f_blk // n_fin

    def first_copy(j):
        cols = pl.ds(pl.multiple_of(2 * j * _LANES, 2 * _LANES), 2 * _LANES)
        return out_copy((pl.ds(0, n_seg), pl.ds(0, 1), pl.ds(0, 8), cols), 1)

    def finish(j, y):
        y = list(y)

        def ffn_steps():
            xb = x_sel.astype(_BF16)
            act = []
            for f in range(f_per):
                gt = _dot(xb, _as_bf16(wg[j * f_per + f]))
                yield
                act.append(gt * jax.nn.sigmoid(gt) * _dot(xb, _as_bf16(wu[j * f_per + f])))
                yield
            yield
            hid = jnp.concatenate(act, axis=1).astype(_BF16)
            rows = pl.ds(pl.multiple_of(j * f_per * 64, 64), f_per * 64)
            for n in range(n_blk):
                y[n] = _dot(hid, _as_bf16(wd[n, rows]), y[n])
                yield

        ffn = ffn_steps()

        def words(r, c, k):
            return jnp.concatenate(
                [wo[2 * j + c, (2 * p + r) * 64:(2 * p + r + 1) * 64] for p in range(k, k + 4)],
                axis=0)

        def prod(f, right, acc):
            for k in range(0, n_pairs, 4):
                left = jnp.concatenate([o0_buf[f, p] for p in range(k, k + 4)], axis=1)
                acc = _dot(_as_bf16(left), right(k).astype(_BF16), acc)
                next(ffn, None)
            return acc

        def put(r, c, a):
            cols = pl.ds(pl.multiple_of((2 * j + c) * _LANES, _LANES), _LANES)
            olds = [acc_buf[(2 * t + r) * 32:(2 * t + r) * 32 + 8, cols] for t in range(n_seg // 2)]
            for t, val in enumerate(olds):
                s = 2 * t + r
                val = val + g_buf[s * 32:s * 32 + 8, :] * a[8 * t:8 * t + 8]
                acc_buf[s * 32:s * 32 + 8, cols] = val
                out_buf[s, 0, :, cols] = val.astype(out_buf.dtype)

        @pl.when(j > 0)
        def _():
            first_copy(j - 1).start()

        _strassen(prod, lambda r, k: _as_bf16(words(r, r, k)),
                  lambda r, c, k: _as_bf16(words(r, c, k)).astype(_F32), put, lambda: None)
        return tuple(y)

    with jax.named_scope('S_finish'):
        y = lax.fori_loop(
            0, n_fin, finish, tuple(jnp.zeros((8, _LANES), _F32) for _ in range(n_blk)))

    order = picked >> (seq.bit_length() - 1)
    bits = jnp.where(order >= 0x8000, order - 0x8000, 0xFFFF - order)
    r_sel = jax.nn.sigmoid(pltpu.bitcast(bits << 16, _F32))
    tokens = [tok_buf[i] for i in range(_TOP_C)]
    out_copy((pl.ds(0, n_seg), pl.ds(1, 3)), 0).wait()
    for j in range(n_fin - 1):
        first_copy(j).wait()
    for i, tok in enumerate(tokens):
        at = pl.ds(tok, 1)
        keep = 1.0 - g_buf[at, :]
        acc_buf[at, :] += jnp.concatenate([keep * (yn * r_sel)[i:i + 1] for yn in y], axis=1)
    for tok in tokens:
        rows = pl.ds(pl.multiple_of((tok >> 3) * 8, 8), 8)
        out_buf[tok >> 5, (tok >> 3) & 3] = acc_buf[rows, :].astype(out_buf.dtype)
    first_copy(n_fin - 1).start()
    patches = []
    for i, tok in enumerate(tokens):
        new = True
        for other in tokens[:i]:
            new = new & ((tok >> 3) != (other >> 3))
        first = ((tok >> 3) & 3) == 0
        at = (pl.ds(tok >> 5, 1), pl.ds((tok >> 3) & 3, 1))
        patches.append((new & ~first, out_copy(at, 0)))
        patches.append((new & first, out_copy(
            at + (pl.ds(0, 8), pl.ds(0, d_model - 2 * _LANES)), 0)))
    for needed, c in patches:
        pl.when(needed)(c.start)
    for needed, c in patches:
        pl.when(needed)(c.wait)
    first_copy(n_fin - 1).wait()


@functools.partial(jax.jit, static_argnames=("A_seg_len",))
def pallas_gated_mix__memory_aug_recurrent_mem_tr__moe_arch_mod__prompt_kernel(
    A_x, A_mem0, A_Wq, A_Wk, A_Wv, A_Wo, A_seg_len,
    B_x, B_w_r, B_w_gate, B_w_up, B_w_down, gate_w,
):
    del B_x
    batch, seq, d_model = A_x.shape
    _, n_heads, d_head = A_Wq.shape
    d_ff = B_w_gate.shape[1]
    assert batch == 1 and A_seg_len == 32 and A_mem0.shape[1] == 8 and d_head == _LANES
    assert seq % 1024 == 0 and seq & (seq - 1) == 0 and d_model == 8 * _LANES
    n_seg = seq // A_seg_len
    n_blk, f_blk = d_model // _LANES, d_ff // _LANES

    hbm = pl.BlockSpec(memory_space=pl.ANY)
    out = pl.pallas_call(
        functools.partial(_kernel, n_seg=n_seg, n_heads=n_heads, d_model=d_model,
                          d_ff=d_ff, scale=d_head ** -0.5),
        out_shape=jax.ShapeDtypeStruct((n_seg, 4, 8, d_model), A_x.dtype),
        in_specs=[hbm] * 11,
        out_specs=hbm,
        scratch_shapes=[
            pltpu.VMEM((n_seg, 4, 8, d_model), A_x.dtype),
            pltpu.VMEM((7, n_seg * 2, d_model // 2), _U32),
            pltpu.VMEM((2, 3, d_model, _LANES), _U32),
            pltpu.VMEM((3, n_heads, d_model // 2, _LANES), _U32),
            pltpu.VMEM((n_blk, n_heads * d_head // 2, _LANES), _U32),
            pltpu.VMEM((f_blk, d_model // 2, _LANES), _U32),
            pltpu.VMEM((f_blk, d_model // 2, _LANES), _U32),
            pltpu.VMEM((n_blk, d_ff // 2, _LANES), _U32),
            pltpu.VMEM((3, n_heads, n_seg * 8, _LANES), _F32),
            pltpu.VMEM((7, n_heads // 2, n_seg * 2, _LANES), _U32),
            pltpu.VMEM((seq, d_model), _F32),
            pltpu.VMEM((seq, _LANES), _F32),
            pltpu.VMEM((n_seg, 4, 8, d_model), A_x.dtype),
            pltpu.VMEM((8, d_model), A_mem0.dtype),
            pltpu.VMEM((n_blk, _LANES), B_w_r.dtype),
            pltpu.VMEM((n_blk, _LANES), gate_w.dtype),
            pltpu.SMEM((n_seg // 4,), jnp.int32),
            pltpu.SemaphoreType.DMA((2, 3)),
            pltpu.SemaphoreType.DMA((2,)),
            pltpu.SemaphoreType.DMA((1,)),
            pltpu.SemaphoreType.DMA((1,)),
            pltpu.SemaphoreType.DMA((1,)),
            pltpu.SemaphoreType.DMA((1,)),
            pltpu.SemaphoreType.DMA((2,)),
        ],
        compiler_params=pltpu.CompilerParams(
            vmem_limit_bytes=120 * 2**20, flags=FLAGS, disable_bounds_checks=True),
        name="gated_rmt_mod",
    )(
        A_x.reshape(n_seg, 4, 8, d_model),
        A_mem0.reshape(8, d_model),
        A_Wq, A_Wk, A_Wv,
        A_Wo.reshape(n_heads * d_head, d_model),
        B_w_r.reshape(n_blk, _LANES), gate_w.reshape(n_blk, _LANES),
        B_w_gate, B_w_up, B_w_down,
    )
    return out.reshape(batch, seq, d_model)
```

```python
import functools

import jax
import jax.numpy as jnp
from jax import lax
import jax.experimental.pallas as pl
import jax.experimental.pallas.tpu as pltpu

_LANES = 128
_TOP_C = 8
_MASKED = -1000000000.0
_KEY_BASE = 0x20000000

_BF16 = jnp.bfloat16
_F32 = jnp.float32
_U32 = jnp.uint32
_CONTRACT_LAST = (((1,), (1,)), ((), ()))


def _as_bf16(words):
    return pltpu.bitcast(words, _BF16)


def _as_words(rows):
    return pltpu.bitcast(rows, _U32)


def _dot(a, b, acc=None):
    y = jnp.dot(a, b, preferred_element_type=_F32)
    return y if acc is None else y + acc


def _iota(shape, dim):
    return lax.broadcasted_iota(jnp.int32, shape, dim)


def _left_factor(i, a):
    return (lambda: a(0, 0) + a(1, 1),
            lambda: a(1, 0) + a(1, 1),
            lambda: a(0, 0),
            lambda: a(1, 1),
            lambda: a(0, 0) + a(0, 1),
            lambda: a(1, 0) - a(0, 0),
            lambda: a(0, 1) - a(1, 1))[i]()


def _block_product(prod, diag, b, put, between):
    m4 = prod(4, lambda *k: diag(1, *k), None)
    m2 = prod(2, lambda *k: b(0, 1, *k) - b(1, 1, *k), None)
    put(0, 1, m2 + m4)
    m1 = prod(1, lambda *k: diag(0, *k), None)
    lower = m2 - m1
    between()
    m3 = prod(3, lambda *k: b(1, 0, *k) - b(0, 0, *k), None)
    put(1, 0, m1 + m3)
    upper = m3 - m4
    m0 = prod(0, lambda *k: b(0, 0, *k) + b(1, 1, *k), None)
    between()
    put(0, 0, prod(6, lambda *k: b(1, 0, *k) + b(1, 1, *k), upper + m0))
    put(1, 1, prod(5, lambda *k: b(0, 0, *k) + b(0, 1, *k), lower + m0))


def _kernel(x_hbm, mem0_hbm, wq_hbm, wk_hbm, wv_hbm, wo_hbm, wr_hbm, gw_hbm,
            wg_hbm, wu_hbm, wd_hbm, out_hbm,
            x_buf, x0_buf, stage, wqkv, wo, wg, wu, wd, qkv0, o0_buf,
            acc_buf, g_buf, out_buf, mem0_buf, wr_buf, gw_buf, tok_buf,
            w_sem, x_sem, x0_sem, wo_sem, ffn_sem, small_sem, out_sem,
            *, n_seg, n_heads, d_model, d_ff, scale):
    n_pairs = n_heads // 2
    n_blk = d_model // _LANES
    f_blk = d_ff // _LANES
    seq = n_seg * 32
    span = n_seg // n_pairs
    half_rows, half_d = n_seg * 4, d_model // 2
    n_keys = seq // (8 * _LANES)
    lane, sub = _iota((8, _LANES), 1), _iota((8, _LANES), 0)

    def w_copy(m, p):
        src = (wq_hbm, wk_hbm, wv_hbm)[m].bitcast(_U32).at[:, p, :]
        return pltpu.make_async_copy(
            src, stage.at[p % 2, m, pl.ds(0, d_model)], w_sem.at[p % 2, m])

    def x_copy(p):
        at = (pl.ds(p * span, span), pl.ds(1, 3))
        return pltpu.make_async_copy(x_hbm.at[at], x_buf.at[at], x_sem.at[p % 2])

    def wo_copy(i):
        rows = n_heads * _LANES // 4
        at, j = pl.ds((i % 2) * rows, rows), i // 2
        cols = pl.ds(pl.multiple_of(j * _LANES, _LANES), _LANES)
        return pltpu.make_async_copy(
            wo_hbm.bitcast(_U32).at[at, cols], wo.at[j, at], wo_sem.at[0])

    def ffn_copy(hbm, dst, j):
        src = hbm.bitcast(_U32).at[:, pl.ds(j * _LANES, _LANES)]
        return pltpu.make_async_copy(src, dst.at[j], ffn_sem.at[0])

    def out_copy(at, sem):
        return pltpu.make_async_copy(out_buf.at[at], out_hbm.at[at], out_sem.at[sem])

    x0_copy = pltpu.make_async_copy(
        x_hbm.at[:, pl.ds(0, 1)], x_buf.at[:, pl.ds(0, 1)], x0_sem.at[0])
    small_copies = [pltpu.make_async_copy(src, dst, small_sem.at[0])
                    for src, dst in ((wr_hbm, wr_buf), (gw_hbm, gw_buf), (mem0_hbm, mem0_buf))]
    ffn_copies = ([ffn_copy(wg_hbm, wg, j) for j in range(f_blk)]
                  + [ffn_copy(wu_hbm, wu, j) for j in range(f_blk)]
                  + [ffn_copy(wd_hbm, wd, j) for j in range(n_blk)])

    def row_dot(xs, w_buf):
        w = w_buf[...].astype(_F32)
        t = xs[:, :_LANES] * w[0:1]
        for j in range(1, n_blk):
            t = t + xs[:, j * _LANES:(j + 1) * _LANES] * w[j:j + 1]
        return jnp.sum(t, axis=1, keepdims=True)

    def gate_and_score(s, scores):
        xs = x_buf[s].reshape(32, d_model).astype(_F32)
        g = jax.nn.sigmoid(row_dot(xs, gw_buf))
        r = row_dot(xs, wr_buf)
        rows = pl.ds(pl.multiple_of(s * 32, 32), 32)
        g_buf[rows, :] = jnp.broadcast_to(g, (32, _LANES))
        acc_buf[rows, :] = (1.0 - g) * xs
        scores = list(scores)
        for b in range(4):
            for u in range(n_keys):
                scores[u] = jnp.where(
                    lane == 4 * s + b - u * _LANES, r[8 * b:8 * b + 8], scores[u])
        return tuple(scores)

    def project_first(m, p, between=lambda: None, left=lambda i: x0_buf[i]):
        def diag(r):
            even, odd = (stage[p % 2, m, pl.ds(r * half_d + t, half_d // 2, stride=2), :]
                         for t in range(2))
            words = ((even & jnp.uint32(0xFFFF)) | (odd << 16),
                     (even >> 16) | (odd & jnp.uint32(0xFFFF0000)))
            for c in range(2):
                wqkv[m, 2 * p + c, r * half_d // 2:(r + 1) * half_d // 2] = words[c]
            return _as_bf16(words[r])

        def block(r, c):
            words = stage[p % 2, m, r * half_d:(r + 1) * half_d]
            return pltpu.bitcast(words & jnp.uint32(0xFFFF0000) if c else words << 16, _F32)

        def prod(i, right, acc):
            return _dot(_as_bf16(left(i)), right().astype(_BF16), acc)

        def put(r, c, val):
            qkv0[m, 2 * p + c, r * half_rows:(r + 1) * half_rows] = val

        _block_product(prod, diag, block, put, between)

    def make_left(i):
        def a(r, c):
            rows = x_buf[r * n_seg // 2:(r + 1) * n_seg // 2, 0, :, c * half_d:(c + 1) * half_d]
            return rows.reshape(half_rows, half_d).astype(_F32)
        words = _as_words(_left_factor(i, a).astype(_BF16))
        x0_buf[i] = words
        return words

    def project_pair(p, mats, scores):
        state = [scores]
        todo = [p * span + t for t in range(span)]

        def between():
            if todo:
                state[0] = gate_and_score(todo.pop(0), state[0])

        while len(todo) > 2 * len(mats):
            between()
        between()
        for m in mats:
            project_first(m, p, between)
        return state[0]

    def fetch(p):
        for m in range(3):
            w_copy(m, p).start()
        x_copy(p).start()

    x0_copy.start()
    w_copy(0, 0).start()
    x0_copy.wait()
    w_copy(1, 0).start()
    w_copy(2, 0).start()
    x_copy(0).start()
    for c in small_copies:
        c.start()
    w_copy(0, 0).wait()
    project_first(0, 0, left=make_left)
    for m in range(3):
        w_copy(m, 1).start()
    w_copy(1, 0).wait()
    project_first(1, 0)
    x_copy(1).start()
    w_copy(2, 0).wait()
    x_copy(0).wait()
    for c in small_copies:
        c.wait()
    scores = project_pair(0, (2,), tuple(jnp.zeros((8, _LANES), _F32) for _ in range(n_keys)))
    fetch(2)
    wo_copy(0).start()
    wo_copy(1).start()

    def prologue(p, scores):
        for m in range(3):
            w_copy(m, p).wait()
        x_copy(p).wait()
        scores = project_pair(p, (0, 1, 2), scores)

        @pl.when(p + 2 < n_pairs)
        def _():
            fetch(p + 2)

        @pl.when(p + 1 < n_pairs)
        def _():
            wo_copy(p + 1).start()

        return scores

    scores = lax.fori_loop(1, n_pairs, prologue, scores)
    for c in ffn_copies:
        c.start()
    for i in range(n_pairs):
        wo_copy(i).wait()

    pad = jnp.zeros((8, _LANES), _F32)

    def segment(s, mem, prev, n_begun, on_pair=None):
        n_q, n_k = (32, 48) if prev is None else (48, 64)
        row, col = _iota((n_q, n_k), 0), _iota((n_q, n_k), 1)
        earlier = (row >= 32) & (row < 40)
        own = (earlier & (col >= 40) & (col < 56)) | (~earlier & (col < 40))
        last = jnp.where(row < 8, 39, jnp.where(row < 32, row + 8,
                                                jnp.where(row < 40, row + 16, row - 32)))
        visible = own & (col <= last)
        hidden = jnp.where(own, _MASKED, -jnp.inf).astype(_F32)

        xs = x_buf[s, 1:4].reshape(24, d_model).astype(_F32)
        full = jnp.concatenate([mem, xs], axis=0)
        h = [full[:, :half_d].astype(_BF16), full[:, half_d:].astype(_BF16)]
        q, k, v, prob, o, o_first, mem_kv = {}, {}, {}, {}, {}, {}, {}

        def weight(m, hd, part):
            return _as_bf16(wqkv[m, hd, part * half_d // 2:(part + 1) * half_d // 2])

        def first(m, hd, seg, rows=8):
            return qkv0[m, hd, pl.ds(pl.multiple_of(seg * 8, 8), rows), :]

        def attend(hd):
            sc = lax.dot_general(q[hd], k[hd], _CONTRACT_LAST, preferred_element_type=_F32)
            sc = jnp.where(visible, sc * scale, hidden)
            ex = jnp.exp(sc - jnp.max(sc, axis=1, keepdims=True))
            total = jnp.sum(ex, axis=1, keepdims=True)
            prob[hd] = (ex * pltpu.reciprocal(total, full_range=False)).astype(_BF16)

        def combine(hd):
            y = _dot(prob[hd], v[hd])
            o[hd] = y[:32].astype(_BF16)
            if prev is not None:
                o_first[hd] = y[32:]
                if on_pair is not None and hd % 2:
                    on_pair(hd // 2, o_first)

        def out_proj(heads, j, acc):
            for hd in heads:
                acc = _dot(o[hd], _as_bf16(wo[j, hd * 64:(hd + 1) * 64, :]), acc)
            return acc

        begun = [[_dot(h[0], weight(m, hd, 0)) for m in range(3)] for hd in range(n_begun)]
        for hd in range(n_heads):
            y = []
            for m in range(3):
                t = begun[hd][m] if hd < n_begun else _dot(h[0], weight(m, hd, 0))
                y.append(_dot(h[1], weight(m, hd, 1), t))
            if hd >= 4 and hd % 4 == 0:
                for u in range(hd - 4, hd):
                    attend(u)
            if hd >= 4 and hd % 4 == 2:
                for u in range(hd - 6, hd - 2):
                    combine(u)
            mem_kv[hd] = (y[1][:8], y[2][:8])
            if prev is not None:
                y[0] = jnp.concatenate([y[0], first(0, hd, s - 1, 16)], axis=0)
            q[hd] = y[0].astype(_BF16)
            for m, dst in ((1, k), (2, v)):
                rows = [y[m][:8], first(m, hd, s), y[m][8:]]
                if prev is not None:
                    rows += [prev[hd][m - 1], first(m, hd, s - 1)]
                dst[hd] = jnp.concatenate(rows + [pad], axis=0).astype(_BF16)

        part = []
        for j in range(n_blk):
            part.append(out_proj(range(n_pairs), j, None))
            if j in (1, 5):
                for u in range(n_heads - 4, n_heads):
                    (attend if j == 1 else combine)(u)
        a = jnp.concatenate(
            [out_proj(range(n_pairs, n_heads), j, part[j]) for j in range(n_blk)], axis=1)
        for b in range(1, 4):
            rows = pl.ds(pl.multiple_of(s * 32 + b * 8, 8), 8)
            t = acc_buf[rows, :] + jnp.tile(g_buf[rows, :], (1, n_blk)) * a[8 * b:8 * b + 8]
            acc_buf[rows, :] = t
            out_buf[s, b] = t.astype(out_buf.dtype)
        return a[:8], (mem_kv if prev is None else o_first)

    keys = []
    for u in range(n_keys):
        r = scores[u].astype(_BF16).astype(_F32)
        bits = lax.shift_right_logical(
            pltpu.bitcast(jnp.where(r == 0.0, 0.0, r), jnp.int32), 16)
        order = jnp.where(bits >= 0x8000, 0xFFFF - bits, bits + 0x8000)
        order = jnp.where(r != r, 0, order)
        token = (lane + u * _LANES) * 8 + sub
        keys.append(pltpu.bitcast(_KEY_BASE + order * seq + (seq - 1 - token), _F32))

    def pick(i, keys, picked, x_sel):
        best = functools.reduce(jnp.maximum, keys)
        best = jnp.max(jnp.max(best, axis=1, keepdims=True), axis=0, keepdims=True)
        keys = tuple(jnp.where(kk == best, 0.0, kk) for kk in keys)
        code = pltpu.bitcast(jnp.broadcast_to(best, (8, _LANES)), jnp.int32) - _KEY_BASE
        tok = seq - 1 - (code[0, 0] & (seq - 1))
        tok_buf[i] = tok
        sub_d = _iota((8, d_model), 0)
        group = x_buf[tok >> 5, (tok >> 3) & 3].astype(_F32)
        one = jnp.sum(jnp.where(sub_d == (tok & 7), group, 0.0), axis=0, keepdims=True)
        return keys, jnp.where(sub == i, code, picked), jnp.where(sub_d == i, one, x_sel)

    def four_segments(i, carry):
        mem, routing = carry
        s = 4 * i
        routing = pick(i, *routing)
        mem, mem_kv = segment(s, mem, None, 0)
        mem, o_a = segment(s + 1, mem, mem_kv, 3)
        mem, mem_kv = segment(s + 2, mem, None, 3)

        def file_pair(p, o_b):
            def a(r, c):
                return jnp.concatenate(
                    [t[2 * p + c][8 * r:8 * r + 8] for t in (o_a, o_b)], axis=0)
            for f in range(7):
                o0_buf[f, p, pl.ds(pl.multiple_of(i * 8, 8), 8), :] = _as_words(
                    _left_factor(f, a).astype(_BF16))

        mem, _ = segment(s + 3, mem, mem_kv, 3, file_pair)
        out_copy((pl.ds(s, 4), pl.ds(1, 3)), 0).start()
        return mem, routing

    routing = (tuple(keys), jnp.zeros((8, _LANES), jnp.int32), jnp.zeros((8, d_model), _F32))
    _, (_, picked, x_sel) = lax.fori_loop(
        0, n_seg // 4, four_segments, (mem0_buf[...].astype(_F32), routing))
    for c in ffn_copies:
        c.wait()

    n_fin = n_blk // 2
    f_per = f_blk // n_fin

    def first_copy(j):
        cols = pl.ds(pl.multiple_of(2 * j * _LANES, 2 * _LANES), 2 * _LANES)
        return out_copy((pl.ds(0, n_seg), pl.ds(0, 1), pl.ds(0, 8), cols), 1)

    def finish(j, y):
        y = list(y)

        def ffn_matmuls():
            xb = x_sel.astype(_BF16)
            act = []
            for f in range(f_per):
                gt = _dot(xb, _as_bf16(wg[j * f_per + f]))
                yield
                act.append(gt * jax.nn.sigmoid(gt) * _dot(xb, _as_bf16(wu[j * f_per + f])))
                yield
            yield
            hid = jnp.concatenate(act, axis=1).astype(_BF16)
            rows = pl.ds(pl.multiple_of(j * f_per * 64, 64), f_per * 64)
            for n in range(n_blk):
                y[n] = _dot(hid, _as_bf16(wd[n, rows]), y[n])
                yield

        ffn = ffn_matmuls()

        def stored(r, c, k):
            return _as_bf16(jnp.concatenate(
                [wo[2 * j + c, (2 * p + r) * 64:(2 * p + r + 1) * 64] for p in range(k, k + 4)],
                axis=0))

        def prod(f, right, acc):
            for k in range(0, n_pairs, 4):
                left = jnp.concatenate([o0_buf[f, p] for p in range(k, k + 4)], axis=1)
                acc = _dot(_as_bf16(left), right(k).astype(_BF16), acc)
                next(ffn, None)
            return acc

        def put(r, c, a):
            cols = pl.ds(pl.multiple_of((2 * j + c) * _LANES, _LANES), _LANES)
            segs = range(r, n_seg, 2)
            rest = [acc_buf[s * 32:s * 32 + 8, cols] for s in segs]
            for t, s in enumerate(segs):
                val = rest[t] + g_buf[s * 32:s * 32 + 8, :] * a[8 * t:8 * t + 8]
                acc_buf[s * 32:s * 32 + 8, cols] = val
                out_buf[s, 0, :, cols] = val.astype(out_buf.dtype)

        @pl.when(j > 0)
        def _():
            first_copy(j - 1).start()

        _block_product(prod, lambda r, k: stored(r, r, k),
                       lambda r, c, k: stored(r, c, k).astype(_F32), put, lambda: None)
        for _ in ffn:
            pass
        return tuple(y)

    y = lax.fori_loop(
        0, n_fin, finish, tuple(jnp.zeros((8, _LANES), _F32) for _ in range(n_blk)))

    order = picked >> (seq.bit_length() - 1)
    bits = jnp.where(order >= 0x8000, order - 0x8000, 0xFFFF - order)
    r_sel = jax.nn.sigmoid(pltpu.bitcast(bits << 16, _F32))
    tokens = [tok_buf[i] for i in range(_TOP_C)]
    out_copy((pl.ds(0, n_seg), pl.ds(1, 3)), 0).wait()
    for j in range(n_fin - 1):
        first_copy(j).wait()
    for i, tok in enumerate(tokens):
        at = pl.ds(tok, 1)
        rest = 1.0 - g_buf[at, :]
        acc_buf[at, :] += jnp.concatenate([rest * (yn * r_sel)[i:i + 1] for yn in y], axis=1)
    for tok in tokens:
        rows = pl.ds(pl.multiple_of((tok >> 3) * 8, 8), 8)
        out_buf[tok >> 5, (tok >> 3) & 3] = acc_buf[rows, :].astype(out_buf.dtype)
    first_copy(n_fin - 1).start()
    patches = []
    for i, tok in enumerate(tokens):
        new = True
        for other in tokens[:i]:
            new = new & ((tok >> 3) != (other >> 3))
        leading = ((tok >> 3) & 3) == 0
        at = (pl.ds(tok >> 5, 1), pl.ds((tok >> 3) & 3, 1))
        patches.append((new & ~leading, out_copy(at, 0)))
        patches.append((new & leading, out_copy(
            at + (pl.ds(0, 8), pl.ds(0, d_model - 2 * _LANES)), 0)))
    for needed, c in patches:
        pl.when(needed)(c.start)
    for needed, c in patches:
        pl.when(needed)(c.wait)
    first_copy(n_fin - 1).wait()


@functools.partial(jax.jit, static_argnames=("A_seg_len",))
def pallas_gated_mix__memory_aug_recurrent_mem_tr__moe_arch_mod__prompt_kernel(
    A_x, A_mem0, A_Wq, A_Wk, A_Wv, A_Wo, A_seg_len,
    B_x, B_w_r, B_w_gate, B_w_up, B_w_down, gate_w,
):
    del B_x
    batch, seq, d_model = A_x.shape
    _, n_heads, d_head = A_Wq.shape
    d_ff = B_w_gate.shape[1]
    assert (batch, A_seg_len, A_mem0.shape[1]) == (1, 32, 8)
    assert (d_model, n_heads, d_head) == (1024, 32, _LANES) and d_ff % 512 == 0
    assert seq >= 1024 and seq & (seq - 1) == 0
    n_seg = seq // A_seg_len
    n_blk, f_blk = d_model // _LANES, d_ff // _LANES

    hbm = pl.BlockSpec(memory_space=pl.ANY)
    dma = pltpu.SemaphoreType.DMA
    out = pl.pallas_call(
        functools.partial(_kernel, n_seg=n_seg, n_heads=n_heads, d_model=d_model,
                          d_ff=d_ff, scale=d_head ** -0.5),
        out_shape=jax.ShapeDtypeStruct((n_seg, 4, 8, d_model), A_x.dtype),
        in_specs=[hbm] * 11,
        out_specs=hbm,
        scratch_shapes=[
            pltpu.VMEM((n_seg, 4, 8, d_model), A_x.dtype),
            pltpu.VMEM((7, n_seg * 2, d_model // 2), _U32),
            pltpu.VMEM((2, 3, d_model + 16, _LANES), _U32),
            pltpu.VMEM((3, n_heads, d_model // 2, _LANES), _U32),
            pltpu.VMEM((n_blk, n_heads * d_head // 2, _LANES), _U32),
            pltpu.VMEM((f_blk, d_model // 2, _LANES), _U32),
            pltpu.VMEM((f_blk, d_model // 2, _LANES), _U32),
            pltpu.VMEM((n_blk, d_ff // 2, _LANES), _U32),
            pltpu.VMEM((3, n_heads, n_seg * 8, _LANES), _F32),
            pltpu.VMEM((7, n_heads // 2, n_seg * 2, _LANES), _U32),
            pltpu.VMEM((seq, d_model), _F32),
            pltpu.VMEM((seq, _LANES), _F32),
            pltpu.VMEM((n_seg, 4, 8, d_model), A_x.dtype),
            pltpu.VMEM((8, d_model), A_mem0.dtype),
            pltpu.VMEM((n_blk, _LANES), B_w_r.dtype),
            pltpu.VMEM((n_blk, _LANES), gate_w.dtype),
            pltpu.SMEM((n_seg // 4,), jnp.int32),
            dma((2, 3)), dma((2,)), dma((1,)), dma((1,)), dma((1,)), dma((1,)), dma((2,)),
        ],
        compiler_params=pltpu.CompilerParams(
            vmem_limit_bytes=120 * 2**20,
            disable_bounds_checks=True,
            flags={"XLA_TPU_EVENLY_DISTRIBUTE_CRITICAL_NODES": True},
        ),
        name="gated_rmt_mod",
    )(
        A_x.reshape(n_seg, 4, 8, d_model),
        A_mem0.reshape(8, d_model),
        A_Wq, A_Wk, A_Wv,
        A_Wo.reshape(n_heads * d_head, d_model),
        B_w_r.reshape(n_blk, _LANES), gate_w.reshape(n_blk, _LANES),
        B_w_gate, B_w_up, B_w_down,
    )
    return out.reshape(batch, seq, d_model)
```

```python
import functools

import jax
import jax.numpy as jnp
from jax import lax
import jax.experimental.pallas as pl
import jax.experimental.pallas.tpu as pltpu

_LANES = 128
_TOP_C = 8
_MASKED = -1000000000.0
_KEY_BASE = 0x20000000

_BF16 = jnp.bfloat16
_F32 = jnp.float32
_U32 = jnp.uint32
_CONTRACT_LAST = (((1,), (1,)), ((), ()))


def _as_bf16(words):
    return pltpu.bitcast(words, _BF16)


def _as_words(rows):
    return pltpu.bitcast(rows, _U32)


def _dot(a, b, acc=None):
    y = jnp.dot(a, b, preferred_element_type=_F32)
    return y if acc is None else y + acc


def _iota(shape, dim):
    return lax.broadcasted_iota(jnp.int32, shape, dim)


def _kernel(x_hbm, mem0_hbm, wq_hbm, wk_hbm, wv_hbm, wo_hbm, wr_hbm, gw_hbm,
            wg_hbm, wu_hbm, wd_hbm, out_hbm,
            x_buf, x0_buf, stage, wqkv, wo, wg, wu, wd, qkv0, o0_buf,
            acc_buf, g_buf, out_buf, mem0_buf, wr_buf, gw_buf, tok_buf,
            w_sem, x_sem, x0_sem, wo_sem, ffn_sem, small_sem, out_sem,
            *, n_seg, n_heads, d_model, d_ff, scale):
    n_pairs = n_heads // 2
    n_blk = d_model // _LANES
    f_blk = d_ff // _LANES
    seq = n_seg * 32
    span = n_seg // n_pairs
    half_d = d_model // 2
    n_keys = seq // (8 * _LANES)
    lane, sub = _iota((8, _LANES), 1), _iota((8, _LANES), 0)

    def w_copy(m, p):
        src = (wq_hbm, wk_hbm, wv_hbm)[m].bitcast(_U32).at[:, p, :]
        return pltpu.make_async_copy(
            src, stage.at[p % 2, m, pl.ds(0, d_model)], w_sem.at[p % 2, m])

    def x_copy(p):
        at = (pl.ds(p * span, span), pl.ds(1, 3))
        return pltpu.make_async_copy(x_hbm.at[at], x_buf.at[at], x_sem.at[p % 2])

    def wo_copy(i):
        rows = n_heads * _LANES // 4
        at, j = pl.ds((i % 2) * rows, rows), i // 2
        cols = pl.ds(pl.multiple_of(j * _LANES, _LANES), _LANES)
        return pltpu.make_async_copy(
            wo_hbm.bitcast(_U32).at[at, cols], wo.at[j, at], wo_sem.at[0])

    def ffn_copy(hbm, dst, j):
        src = hbm.bitcast(_U32).at[:, pl.ds(j * _LANES, _LANES)]
        return pltpu.make_async_copy(src, dst.at[j], ffn_sem.at[0])

    def out_copy(at, sem):
        return pltpu.make_async_copy(out_buf.at[at], out_hbm.at[at], out_sem.at[sem])

    x0_copy = pltpu.make_async_copy(
        x_hbm.at[:, pl.ds(0, 1)], x_buf.at[:, pl.ds(0, 1)], x0_sem.at[0])
    small_copies = [pltpu.make_async_copy(src, dst, small_sem.at[0])
                    for src, dst in ((wr_hbm, wr_buf), (gw_hbm, gw_buf), (mem0_hbm, mem0_buf))]
    ffn_copies = ([ffn_copy(wg_hbm, wg, j) for j in range(f_blk)]
                  + [ffn_copy(wu_hbm, wu, j) for j in range(f_blk)]
                  + [ffn_copy(wd_hbm, wd, j) for j in range(n_blk)])

    def row_dot(xs, w_buf):
        w = w_buf[...].astype(_F32)
        t = xs[:, :_LANES] * w[0:1]
        for j in range(1, n_blk):
            t = t + xs[:, j * _LANES:(j + 1) * _LANES] * w[j:j + 1]
        return jnp.sum(t, axis=1, keepdims=True)

    def gate_and_score(s, scores):
        xs = x_buf[s].reshape(32, d_model).astype(_F32)
        g = jax.nn.sigmoid(row_dot(xs, gw_buf))
        r = row_dot(xs, wr_buf)
        rows = pl.ds(pl.multiple_of(s * 32, 32), 32)
        g_buf[rows, :] = jnp.broadcast_to(g, (32, _LANES))
        acc_buf[rows, :] = (1.0 - g) * xs
        scores = list(scores)
        for b in range(4):
            for u in range(n_keys):
                scores[u] = jnp.where(
                    lane == 4 * s + b - u * _LANES, r[8 * b:8 * b + 8], scores[u])
        return tuple(scores)

    def project_first(m, p, between=lambda: None):
        even, odd = (stage[p % 2, m, pl.ds(t, half_d, stride=2), :] for t in range(2))
        words = ((even & jnp.uint32(0xFFFF)) | (odd << 16),
                 (even >> 16) | (odd & jnp.uint32(0xFFFF0000)))
        for c in range(2):
            wqkv[m, 2 * p + c] = words[c]
        for c in range(2):
            qkv0[m, 2 * p + c] = _dot(_as_bf16(x0_buf[...]), _as_bf16(words[c]))
            between()

    def project_pair(p, mats, scores):
        state = [scores]
        todo = [p * span + t for t in range(span)]

        def between():
            if todo:
                state[0] = gate_and_score(todo.pop(0), state[0])

        while len(todo) > 2 * len(mats):
            between()
        between()
        for m in mats:
            project_first(m, p, between)
        return state[0]

    def fetch(p):
        for m in range(3):
            w_copy(m, p).start()
        x_copy(p).start()

    x0_copy.start()
    w_copy(0, 0).start()
    x0_copy.wait()
    w_copy(1, 0).start()
    w_copy(2, 0).start()
    x_copy(0).start()
    for c in small_copies:
        c.start()
    x0_buf[...] = _as_words(x_buf[:, 0].reshape(n_seg * 8, d_model))
    w_copy(0, 0).wait()
    project_first(0, 0)
    for m in range(3):
        w_copy(m, 1).start()
    w_copy(1, 0).wait()
    project_first(1, 0)
    x_copy(1).start()
    w_copy(2, 0).wait()
    x_copy(0).wait()
    for c in small_copies:
        c.wait()
    scores = project_pair(0, (2,), tuple(jnp.zeros((8, _LANES), _F32) for _ in range(n_keys)))
    fetch(2)
    wo_copy(0).start()
    wo_copy(1).start()

    def prologue(p, scores):
        for m in range(3):
            w_copy(m, p).wait()
        x_copy(p).wait()
        scores = project_pair(p, (0, 1, 2), scores)

        @pl.when(p + 2 < n_pairs)
        def _():
            fetch(p + 2)

        @pl.when(p + 1 < n_pairs)
        def _():
            wo_copy(p + 1).start()

        return scores

    scores = lax.fori_loop(1, n_pairs, prologue, scores)
    for c in ffn_copies:
        c.start()
    for i in range(n_pairs):
        wo_copy(i).wait()

    pad = jnp.zeros((8, _LANES), _F32)

    def segment(s, mem, prev, n_begun):
        n_q, n_k = (32, 48) if prev is None else (48, 64)
        row, col = _iota((n_q, n_k), 0), _iota((n_q, n_k), 1)
        earlier = (row >= 32) & (row < 40)
        own = (earlier & (col >= 40) & (col < 56)) | (~earlier & (col < 40))
        last = jnp.where(row < 8, 39, jnp.where(row < 32, row + 8,
                                                jnp.where(row < 40, row + 16, row - 32)))
        visible = own & (col <= last)
        hidden = jnp.where(own, _MASKED, -jnp.inf).astype(_F32)

        xs = x_buf[s, 1:4].reshape(24, d_model).astype(_F32)
        full = jnp.concatenate([mem, xs], axis=0)
        h = [full[:, :half_d].astype(_BF16), full[:, half_d:].astype(_BF16)]
        q, k, v, prob, o, mem_kv = {}, {}, {}, {}, {}, {}

        def weight(m, hd, part):
            return _as_bf16(wqkv[m, hd, part * half_d // 2:(part + 1) * half_d // 2])

        def first(m, hd, seg, rows=8):
            return qkv0[m, hd, pl.ds(pl.multiple_of(seg * 8, 8), rows), :]

        def attend(hd):
            sc = lax.dot_general(q[hd], k[hd], _CONTRACT_LAST, preferred_element_type=_F32)
            sc = jnp.where(visible, sc * scale, hidden)
            ex = jnp.exp(sc - jnp.max(sc, axis=1, keepdims=True))
            total = jnp.sum(ex, axis=1, keepdims=True)
            prob[hd] = (ex * pltpu.reciprocal(total, full_range=False)).astype(_BF16)

        def combine(hd):
            y = _dot(prob[hd], v[hd])
            o[hd] = y[:32].astype(_BF16)
            if prev is not None:
                words = pl.ds(pl.multiple_of((s - 1) * 4, 8), 8)
                o0_buf[hd, words, :] = _as_words(y[32:].astype(_BF16))

        def out_proj(heads, j, acc):
            for hd in heads:
                acc = _dot(o[hd], _as_bf16(wo[j, hd * 64:(hd + 1) * 64, :]), acc)
            return acc

        begun = [[_dot(h[0], weight(m, hd, 0)) for m in range(3)] for hd in range(n_begun)]
        for hd in range(n_heads):
            y = []
            for m in range(3):
                t = begun[hd][m] if hd < n_begun else _dot(h[0], weight(m, hd, 0))
                y.append(_dot(h[1], weight(m, hd, 1), t))
            if hd >= 4 and hd % 4 == 0:
                for u in range(hd - 4, hd):
                    attend(u)
            if hd >= 4 and hd % 4 == 2:
                for u in range(hd - 6, hd - 2):
                    combine(u)
            mem_kv[hd] = (y[1][:8], y[2][:8])
            if prev is not None:
                y[0] = jnp.concatenate([y[0], first(0, hd, s - 1, 16)], axis=0)
            q[hd] = y[0].astype(_BF16)
            for m, dst in ((1, k), (2, v)):
                rows = [y[m][:8], first(m, hd, s), y[m][8:]]
                if prev is not None:
                    rows += [prev[hd][m - 1], first(m, hd, s - 1)]
                dst[hd] = jnp.concatenate(rows + [pad], axis=0).astype(_BF16)

        part = []
        for j in range(n_blk):
            part.append(out_proj(range(n_pairs), j, None))
            if j in (1, 5):
                for u in range(n_heads - 4, n_heads):
                    (attend if j == 1 else combine)(u)
        a = jnp.concatenate(
            [out_proj(range(n_pairs, n_heads), j, part[j]) for j in range(n_blk)], axis=1)
        for b in range(1, 4):
            rows = pl.ds(pl.multiple_of(s * 32 + b * 8, 8), 8)
            t = acc_buf[rows, :] + jnp.tile(g_buf[rows, :], (1, n_blk)) * a[8 * b:8 * b + 8]
            acc_buf[rows, :] = t
            out_buf[s, b] = t.astype(out_buf.dtype)
        return a[:8], mem_kv

    keys = []
    for u in range(n_keys):
        r = scores[u].astype(_BF16).astype(_F32)
        bits = lax.shift_right_logical(
            pltpu.bitcast(jnp.where(r == 0.0, 0.0, r), jnp.int32), 16)
        order = jnp.where(bits >= 0x8000, 0xFFFF - bits, bits + 0x8000)
        order = jnp.where(r != r, 0, order)
        token = (lane + u * _LANES) * 8 + sub
        keys.append(pltpu.bitcast(_KEY_BASE + order * seq + (seq - 1 - token), _F32))

    def pick(i, keys, picked, x_sel):
        best = functools.reduce(jnp.maximum, keys)
        best = jnp.max(jnp.max(best, axis=1, keepdims=True), axis=0, keepdims=True)
        keys = tuple(jnp.where(kk == best, 0.0, kk) for kk in keys)
        code = pltpu.bitcast(jnp.broadcast_to(best, (8, _LANES)), jnp.int32) - _KEY_BASE
        tok = seq - 1 - (code[0, 0] & (seq - 1))
        tok_buf[i] = tok
        sub_d = _iota((8, d_model), 0)
        group = x_buf[tok >> 5, (tok >> 3) & 3].astype(_F32)
        one = jnp.sum(jnp.where(sub_d == (tok & 7), group, 0.0), axis=0, keepdims=True)
        return keys, jnp.where(sub == i, code, picked), jnp.where(sub_d == i, one, x_sel)

    def four_segments(i, carry):
        mem, routing = carry
        s = 4 * i
        routing = pick(i, *routing)
        mem, mem_kv = segment(s, mem, None, 0)
        mem, _ = segment(s + 1, mem, mem_kv, 3)
        mem, mem_kv = segment(s + 2, mem, None, 3)
        mem, _ = segment(s + 3, mem, mem_kv, 3)
        out_copy((pl.ds(s, 4), pl.ds(1, 3)), 0).start()
        return mem, routing

    routing = (tuple(keys), jnp.zeros((8, _LANES), jnp.int32), jnp.zeros((8, d_model), _F32))
    _, (_, picked, x_sel) = lax.fori_loop(
        0, n_seg // 4, four_segments, (mem0_buf[...].astype(_F32), routing))
    for c in ffn_copies:
        c.wait()

    n_fin = n_blk // 2
    f_per = f_blk // n_fin

    def first_copy(j):
        cols = pl.ds(pl.multiple_of(2 * j * _LANES, 2 * _LANES), 2 * _LANES)
        return out_copy((pl.ds(0, n_seg), pl.ds(0, 1), pl.ds(0, 8), cols), 1)

    def finish(j, y):
        y = list(y)

        def ffn_matmuls():
            xb = x_sel.astype(_BF16)
            act = []
            for f in range(f_per):
                gt = _dot(xb, _as_bf16(wg[j * f_per + f]))
                yield
                act.append(gt * jax.nn.sigmoid(gt) * _dot(xb, _as_bf16(wu[j * f_per + f])))
                yield
            yield
            hid = jnp.concatenate(act, axis=1).astype(_BF16)
            rows = pl.ds(pl.multiple_of(j * f_per * 64, 64), f_per * 64)
            for n in range(n_blk):
                y[n] = _dot(hid, _as_bf16(wd[n, rows]), y[n])
                yield

        ffn = ffn_matmuls()

        @pl.when(j > 0)
        def _():
            first_copy(j - 1).start()

        for c in range(2):
            cols = pl.ds(pl.multiple_of((2 * j + c) * _LANES, _LANES), _LANES)
            for segs in (range(n_seg // 2), range(n_seg // 2, n_seg)):
                words = pl.ds(segs[0] * 4, len(segs) * 4)
                a = None
                for hd in range(0, n_heads, 4):
                    left = jnp.concatenate(
                        [o0_buf[u, words, :] for u in range(hd, hd + 4)], axis=1)
                    a = _dot(_as_bf16(left), _as_bf16(wo[2 * j + c, hd * 64:(hd + 4) * 64]), a)
                    next(ffn, None)
                rest = [acc_buf[s * 32:s * 32 + 8, cols] for s in segs]
                for t, s in enumerate(segs):
                    val = rest[t] + g_buf[s * 32:s * 32 + 8, :] * a[8 * t:8 * t + 8]
                    acc_buf[s * 32:s * 32 + 8, cols] = val
                    out_buf[s, 0, :, cols] = val.astype(out_buf.dtype)
        for _ in ffn:
            pass
        return tuple(y)

    y = lax.fori_loop(
        0, n_fin, finish, tuple(jnp.zeros((8, _LANES), _F32) for _ in range(n_blk)))

    order = picked >> (seq.bit_length() - 1)
    bits = jnp.where(order >= 0x8000, order - 0x8000, 0xFFFF - order)
    r_sel = jax.nn.sigmoid(pltpu.bitcast(bits << 16, _F32))
    tokens = [tok_buf[i] for i in range(_TOP_C)]
    out_copy((pl.ds(0, n_seg), pl.ds(1, 3)), 0).wait()
    for j in range(n_fin - 1):
        first_copy(j).wait()
    for i, tok in enumerate(tokens):
        at = pl.ds(tok, 1)
        rest = 1.0 - g_buf[at, :]
        acc_buf[at, :] += jnp.concatenate([rest * (yn * r_sel)[i:i + 1] for yn in y], axis=1)
    for tok in tokens:
        rows = pl.ds(pl.multiple_of((tok >> 3) * 8, 8), 8)
        out_buf[tok >> 5, (tok >> 3) & 3] = acc_buf[rows, :].astype(out_buf.dtype)
    first_copy(n_fin - 1).start()
    patches = []
    for i, tok in enumerate(tokens):
        new = True
        for other in tokens[:i]:
            new = new & ((tok >> 3) != (other >> 3))
        leading = ((tok >> 3) & 3) == 0
        at = (pl.ds(tok >> 5, 1), pl.ds((tok >> 3) & 3, 1))
        patches.append((new & ~leading, out_copy(at, 0)))
        patches.append((new & leading, out_copy(
            at + (pl.ds(0, 8), pl.ds(0, d_model - 2 * _LANES)), 0)))
    for needed, c in patches:
        pl.when(needed)(c.start)
    for needed, c in patches:
        pl.when(needed)(c.wait)
    first_copy(n_fin - 1).wait()


@functools.partial(jax.jit, static_argnames=("A_seg_len",))
def pallas_gated_mix__memory_aug_recurrent_mem_tr__moe_arch_mod__prompt_kernel(
    A_x, A_mem0, A_Wq, A_Wk, A_Wv, A_Wo, A_seg_len,
    B_x, B_w_r, B_w_gate, B_w_up, B_w_down, gate_w,
):
    del B_x
    batch, seq, d_model = A_x.shape
    _, n_heads, d_head = A_Wq.shape
    d_ff = B_w_gate.shape[1]
    assert (batch, A_seg_len, A_mem0.shape[1]) == (1, 32, 8)
    assert (d_model, n_heads, d_head) == (1024, 32, _LANES) and d_ff % 512 == 0
    assert seq >= 1024 and seq & (seq - 1) == 0
    n_seg = seq // A_seg_len
    n_blk, f_blk = d_model // _LANES, d_ff // _LANES

    hbm = pl.BlockSpec(memory_space=pl.ANY)
    dma = pltpu.SemaphoreType.DMA
    out = pl.pallas_call(
        functools.partial(_kernel, n_seg=n_seg, n_heads=n_heads, d_model=d_model,
                          d_ff=d_ff, scale=d_head ** -0.5),
        out_shape=jax.ShapeDtypeStruct((n_seg, 4, 8, d_model), A_x.dtype),
        in_specs=[hbm] * 11,
        out_specs=hbm,
        scratch_shapes=[
            pltpu.VMEM((n_seg, 4, 8, d_model), A_x.dtype),
            pltpu.VMEM((n_seg * 4, d_model), _U32),
            pltpu.VMEM((2, 3, d_model + 16, _LANES), _U32),
            pltpu.VMEM((3, n_heads, d_model // 2, _LANES), _U32),
            pltpu.VMEM((n_blk, n_heads * d_head // 2, _LANES), _U32),
            pltpu.VMEM((f_blk, d_model // 2, _LANES), _U32),
            pltpu.VMEM((f_blk, d_model // 2, _LANES), _U32),
            pltpu.VMEM((n_blk, d_ff // 2, _LANES), _U32),
            pltpu.VMEM((3, n_heads, n_seg * 8, _LANES), _F32),
            pltpu.VMEM((n_heads, n_seg * 4, _LANES), _U32),
            pltpu.VMEM((seq, d_model), _F32),
            pltpu.VMEM((seq, _LANES), _F32),
            pltpu.VMEM((n_seg, 4, 8, d_model), A_x.dtype),
            pltpu.VMEM((8, d_model), A_mem0.dtype),
            pltpu.VMEM((n_blk, _LANES), B_w_r.dtype),
            pltpu.VMEM((n_blk, _LANES), gate_w.dtype),
            pltpu.SMEM((n_seg // 4,), jnp.int32),
            dma((2, 3)), dma((2,)), dma((1,)), dma((1,)), dma((1,)), dma((1,)), dma((2,)),
        ],
        compiler_params=pltpu.CompilerParams(
            vmem_limit_bytes=120 * 2**20,
            disable_bounds_checks=True,
            flags={"XLA_TPU_EVENLY_DISTRIBUTE_CRITICAL_NODES": True},
        ),
        name="gated_rmt_mod",
    )(
        A_x.reshape(n_seg, 4, 8, d_model),
        A_mem0.reshape(8, d_model),
        A_Wq, A_Wk, A_Wv,
        A_Wo.reshape(n_heads * d_head, d_model),
        B_w_r.reshape(n_blk, _LANES), gate_w.reshape(n_blk, _LANES),
        B_w_gate, B_w_up, B_w_down,
    )
    return out.reshape(batch, seq, d_model)
```

```python
import functools

import jax
import jax.numpy as jnp
from jax import lax
import jax.experimental.pallas as pl
import jax.experimental.pallas.tpu as pltpu

_LANES = 128
_TOP_C = 8
_MASKED = -1000000000.0
_KEY_BASE = 0x20000000

_BF16 = jnp.bfloat16
_F32 = jnp.float32
_U32 = jnp.uint32
_CONTRACT_LAST = (((1,), (1,)), ((), ()))


def _as_bf16(words):
    return pltpu.bitcast(words, _BF16)


def _as_words(rows):
    return pltpu.bitcast(rows, _U32)


def _dot(a, b, acc=None):
    y = jnp.dot(a, b, preferred_element_type=_F32)
    return y if acc is None else y + acc


def _iota(shape, dim):
    return lax.broadcasted_iota(jnp.int32, shape, dim)


def _kernel(x_hbm, mem0_hbm, wq_hbm, wk_hbm, wv_hbm, wo_hbm, wr_hbm, gw_hbm,
            wg_hbm, wu_hbm, wd_hbm, out_hbm,
            x_buf, x0_buf, stage, wqkv, wo, wg, wu, wd, qkv0, o0_buf,
            acc_buf, g_buf, out_buf, mem0_buf, wr_buf, gw_buf, tok_buf,
            w_sem, x_sem, x0_sem, wo_sem, ffn_sem, small_sem, out_sem,
            *, n_seg, n_heads, d_model, d_ff, scale):
    n_pairs = n_heads // 2
    n_blk = d_model // _LANES
    f_blk = d_ff // _LANES
    seq = n_seg * 32
    span = n_seg // n_pairs
    half_d = d_model // 2
    n_keys = seq // (8 * _LANES)
    lane, sub = _iota((8, _LANES), 1), _iota((8, _LANES), 0)

    def w_copy(m, p):
        src = (wq_hbm, wk_hbm, wv_hbm)[m].bitcast(_U32).at[:, p, :]
        return pltpu.make_async_copy(
            src, stage.at[p % 2, m, pl.ds(0, d_model)], w_sem.at[p % 2, m])

    def x0_copy(t):
        at = (pl.ds(t * n_seg // 2, n_seg // 2), pl.ds(0, 1))
        return pltpu.make_async_copy(x_hbm.at[at], x_buf.at[at], x0_sem.at[t])

    def x_copy(p):
        at = (pl.ds(p * span, span), pl.ds(1, 3))
        return pltpu.make_async_copy(x_hbm.at[at], x_buf.at[at], x_sem.at[p % 2])

    def wo_copy(i):
        rows = n_heads * _LANES // 4
        at, j = pl.ds((i % 2) * rows, rows), i // 2
        cols = pl.ds(pl.multiple_of(j * _LANES, _LANES), _LANES)
        return pltpu.make_async_copy(
            wo_hbm.bitcast(_U32).at[at, cols], wo.at[j, at], wo_sem.at[0])

    def ffn_copy(hbm, dst, j):
        src = hbm.bitcast(_U32).at[:, pl.ds(j * _LANES, _LANES)]
        return pltpu.make_async_copy(src, dst.at[j], ffn_sem.at[0])

    def out_copy(at, sem):
        return pltpu.make_async_copy(out_buf.at[at], out_hbm.at[at], out_sem.at[sem])

    small_copies = [pltpu.make_async_copy(src, dst, small_sem.at[0])
                    for src, dst in ((wr_hbm, wr_buf), (gw_hbm, gw_buf), (mem0_hbm, mem0_buf))]
    ffn_copies = ([ffn_copy(wg_hbm, wg, j) for j in range(f_blk)]
                  + [ffn_copy(wu_hbm, wu, j) for j in range(f_blk)]
                  + [ffn_copy(wd_hbm, wd, j) for j in range(n_blk)])

    def row_dot(xs, w_buf):
        w = w_buf[...].astype(_F32)
        t = xs[:, :_LANES] * w[0:1]
        for j in range(1, n_blk):
            t = t + xs[:, j * _LANES:(j + 1) * _LANES] * w[j:j + 1]
        return jnp.sum(t, axis=1, keepdims=True)

    def gate_and_score(s, scores):
        xs = x_buf[s].reshape(32, d_model).astype(_F32)
        g = jax.nn.sigmoid(row_dot(xs, gw_buf))
        r = row_dot(xs, wr_buf)
        rows = pl.ds(pl.multiple_of(s * 32, 32), 32)
        g_buf[rows, :] = jnp.broadcast_to(g, (32, _LANES))
        acc_buf[rows, :] = (1.0 - g) * xs
        scores = list(scores)
        for b in range(4):
            for u in range(n_keys):
                scores[u] = jnp.where(
                    lane == 4 * s + b - u * _LANES, r[8 * b:8 * b + 8], scores[u])
        return tuple(scores)

    def regroup(m, p):
        even, odd = (stage[p % 2, m, pl.ds(t, half_d, stride=2), :] for t in range(2))
        words = ((even & jnp.uint32(0xFFFF)) | (odd << 16),
                 (even >> 16) | (odd & jnp.uint32(0xFFFF0000)))
        for c in range(2):
            wqkv[m, 2 * p + c] = words[c]
        return words

    def project_first(m, p, between=lambda: None):
        words = regroup(m, p)
        for c in range(2):
            qkv0[m, 2 * p + c] = _dot(_as_bf16(x0_buf[...]), _as_bf16(words[c]))
            between()

    def project_pair(p, mats, scores):
        state = [scores]
        todo = [p * span + t for t in range(span)]

        def between():
            if todo:
                state[0] = gate_and_score(todo.pop(0), state[0])

        while len(todo) > 2 * len(mats):
            between()
        between()
        for m in mats:
            project_first(m, p, between)
        return state[0]

    def fetch(p):
        for m in range(3):
            w_copy(m, p).start()
        x_copy(p).start()

    def first_half(t, words):
        rows = x_buf[t * n_seg // 2:(t + 1) * n_seg // 2, 0].reshape(n_seg * 4, d_model)
        x0_buf[t * n_seg * 2:(t + 1) * n_seg * 2] = _as_words(rows)
        for c in range(2):
            qkv0[0, c, t * n_seg * 4:(t + 1) * n_seg * 4] = _dot(rows, _as_bf16(words[c]))

    w_copy(0, 0).start()
    x0_copy(0).start()
    x0_copy(1).start()
    x0_copy(0).wait()
    w_copy(0, 0).wait()
    w_copy(1, 0).start()
    first_half(0, regroup(0, 0))
    w_copy(2, 0).start()
    x_copy(0).start()
    for c in small_copies:
        c.start()
    x0_copy(1).wait()
    first_half(1, (wqkv[0, 0], wqkv[0, 1]))
    for m in range(3):
        w_copy(m, 1).start()
    w_copy(1, 0).wait()
    project_first(1, 0)
    x_copy(1).start()
    w_copy(2, 0).wait()
    x_copy(0).wait()
    for c in small_copies:
        c.wait()
    scores = project_pair(0, (2,), tuple(jnp.zeros((8, _LANES), _F32) for _ in range(n_keys)))
    fetch(2)
    wo_copy(0).start()
    wo_copy(1).start()

    def prologue(p, scores):
        for m in range(3):
            w_copy(m, p).wait()
        x_copy(p).wait()
        scores = project_pair(p, (0, 1, 2), scores)

        @pl.when(p + 2 < n_pairs)
        def _():
            fetch(p + 2)

        @pl.when(p + 1 < n_pairs)
        def _():
            wo_copy(p + 1).start()

        return scores

    scores = lax.fori_loop(1, n_pairs, prologue, scores)
    for c in ffn_copies:
        c.start()
    for i in range(n_pairs):
        wo_copy(i).wait()

    pad = jnp.zeros((8, _LANES), _F32)

    def segment(s, mem, prev, n_begun):
        n_q, n_k = (32, 48) if prev is None else (48, 64)
        row, col = _iota((n_q, n_k), 0), _iota((n_q, n_k), 1)
        earlier = (row >= 32) & (row < 40)
        own = (earlier & (col >= 40) & (col < 56)) | (~earlier & (col < 40))
        last = jnp.where(row < 8, 39, jnp.where(row < 32, row + 8,
                                                jnp.where(row < 40, row + 16, row - 32)))
        visible = own & (col <= last)
        hidden = jnp.where(own, _MASKED, -jnp.inf).astype(_F32)

        xs = x_buf[s, 1:4].reshape(24, d_model).astype(_F32)
        full = jnp.concatenate([mem, xs], axis=0)
        h = [full[:, :half_d].astype(_BF16), full[:, half_d:].astype(_BF16)]
        q, k, v, prob, o, mem_kv = {}, {}, {}, {}, {}, {}

        def weight(m, hd, part):
            return _as_bf16(wqkv[m, hd, part * half_d // 2:(part + 1) * half_d // 2])

        def first(m, hd, seg, rows=8):
            return qkv0[m, hd, pl.ds(pl.multiple_of(seg * 8, 8), rows), :]

        def attend(hd):
            sc = lax.dot_general(q[hd], k[hd], _CONTRACT_LAST, preferred_element_type=_F32)
            sc = jnp.where(visible, sc * scale, hidden)
            ex = jnp.exp(sc - jnp.max(sc, axis=1, keepdims=True))
            total = jnp.sum(ex, axis=1, keepdims=True)
            prob[hd] = (ex * pltpu.reciprocal(total, full_range=False)).astype(_BF16)

        def combine(hd):
            y = _dot(prob[hd], v[hd])
            o[hd] = y[:32].astype(_BF16)
            if prev is not None:
                words = pl.ds(pl.multiple_of((s - 1) * 4, 8), 8)
                o0_buf[hd, words, :] = _as_words(y[32:].astype(_BF16))

        def out_proj(heads, j, acc):
            for hd in heads:
                acc = _dot(o[hd], _as_bf16(wo[j, hd * 64:(hd + 1) * 64, :]), acc)
            return acc

        begun = [[_dot(h[0], weight(m, hd, 0)) for m in range(3)] for hd in range(n_begun)]
        for hd in range(n_heads):
            y = []
            for m in range(3):
                t = begun[hd][m] if hd < n_begun else _dot(h[0], weight(m, hd, 0))
                y.append(_dot(h[1], weight(m, hd, 1), t))
            if hd >= 4 and hd % 4 == 0:
                for u in range(hd - 4, hd):
                    attend(u)
            if hd >= 4 and hd % 4 == 2:
                for u in range(hd - 6, hd - 2):
                    combine(u)
            mem_kv[hd] = (y[1][:8], y[2][:8])
            if prev is not None:
                y[0] = jnp.concatenate([y[0], first(0, hd, s - 1, 16)], axis=0)
            q[hd] = y[0].astype(_BF16)
            for m, dst in ((1, k), (2, v)):
                rows = [y[m][:8], first(m, hd, s), y[m][8:]]
                if prev is not None:
                    rows += [prev[hd][m - 1], first(m, hd, s - 1)]
                dst[hd] = jnp.concatenate(rows + [pad], axis=0).astype(_BF16)

        part = []
        for j in range(n_blk):
            part.append(out_proj(range(n_pairs), j, None))
            if j in (1, 5):
                for u in range(n_heads - 4, n_heads):
                    (attend if j == 1 else combine)(u)
        a = jnp.concatenate(
            [out_proj(range(n_pairs, n_heads), j, part[j]) for j in range(n_blk)], axis=1)
        for b in range(1, 4):
            rows = pl.ds(pl.multiple_of(s * 32 + b * 8, 8), 8)
            t = acc_buf[rows, :] + jnp.tile(g_buf[rows, :], (1, n_blk)) * a[8 * b:8 * b + 8]
            acc_buf[rows, :] = t
            out_buf[s, b] = t.astype(out_buf.dtype)
        return a[:8], mem_kv

    keys = []
    for u in range(n_keys):
        r = scores[u].astype(_BF16).astype(_F32)
        bits = lax.shift_right_logical(
            pltpu.bitcast(jnp.where(r == 0.0, 0.0, r), jnp.int32), 16)
        order = jnp.where(bits >= 0x8000, 0xFFFF - bits, bits + 0x8000)
        order = jnp.where(r != r, 0, order)
        token = (lane + u * _LANES) * 8 + sub
        keys.append(pltpu.bitcast(_KEY_BASE + order * seq + (seq - 1 - token), _F32))

    def pick(i, keys, picked, x_sel):
        best = functools.reduce(jnp.maximum, keys)
        best = jnp.max(jnp.max(best, axis=1, keepdims=True), axis=0, keepdims=True)
        keys = tuple(jnp.where(kk == best, 0.0, kk) for kk in keys)
        code = pltpu.bitcast(jnp.broadcast_to(best, (8, _LANES)), jnp.int32) - _KEY_BASE
        tok = seq - 1 - (code[0, 0] & (seq - 1))
        tok_buf[i] = tok
        sub_d = _iota((8, d_model), 0)
        group = x_buf[tok >> 5, (tok >> 3) & 3].astype(_F32)
        one = jnp.sum(jnp.where(sub_d == (tok & 7), group, 0.0), axis=0, keepdims=True)
        return keys, jnp.where(sub == i, code, picked), jnp.where(sub_d == i, one, x_sel)

    def four_segments(i, carry):
        mem, routing = carry
        s = 4 * i
        routing = pick(i, *routing)
        mem, mem_kv = segment(s, mem, None, 0)
        mem, _ = segment(s + 1, mem, mem_kv, 3)
        mem, mem_kv = segment(s + 2, mem, None, 3)
        mem, _ = segment(s + 3, mem, mem_kv, 3)
        out_copy((pl.ds(s, 4), pl.ds(1, 3)), 0).start()
        return mem, routing

    routing = (tuple(keys), jnp.zeros((8, _LANES), jnp.int32), jnp.zeros((8, d_model), _F32))
    _, (_, picked, x_sel) = lax.fori_loop(
        0, n_seg // 4, four_segments, (mem0_buf[...].astype(_F32), routing))
    for c in ffn_copies:
        c.wait()

    n_fin = n_blk // 2
    f_per = f_blk // n_fin

    def first_copy(j):
        cols = pl.ds(pl.multiple_of(2 * j * _LANES, 2 * _LANES), 2 * _LANES)
        return out_copy((pl.ds(0, n_seg), pl.ds(0, 1), pl.ds(0, 8), cols), 1)

    def finish(j, y):
        y = list(y)

        def ffn_matmuls():
            xb = x_sel.astype(_BF16)
            act = []
            for f in range(f_per):
                gt = _dot(xb, _as_bf16(wg[j * f_per + f]))
                yield
                act.append(gt * jax.nn.sigmoid(gt) * _dot(xb, _as_bf16(wu[j * f_per + f])))
                yield
            yield
            hid = jnp.concatenate(act, axis=1).astype(_BF16)
            rows = pl.ds(pl.multiple_of(j * f_per * 64, 64), f_per * 64)
            for n in range(n_blk):
                y[n] = _dot(hid, _as_bf16(wd[n, rows]), y[n])
                yield

        ffn = ffn_matmuls()

        @pl.when(j > 0)
        def _():
            first_copy(j - 1).start()

        for c in range(2):
            cols = pl.ds(pl.multiple_of((2 * j + c) * _LANES, _LANES), _LANES)
            for segs in (range(n_seg // 2), range(n_seg // 2, n_seg)):
                words = pl.ds(segs[0] * 4, len(segs) * 4)
                a = None
                for hd in range(0, n_heads, 4):
                    left = jnp.concatenate(
                        [o0_buf[u, words, :] for u in range(hd, hd + 4)], axis=1)
                    a = _dot(_as_bf16(left), _as_bf16(wo[2 * j + c, hd * 64:(hd + 4) * 64]), a)
                    next(ffn, None)
                rest = [acc_buf[s * 32:s * 32 + 8, cols] for s in segs]
                for t, s in enumerate(segs):
                    val = rest[t] + g_buf[s * 32:s * 32 + 8, :] * a[8 * t:8 * t + 8]
                    acc_buf[s * 32:s * 32 + 8, cols] = val
                    out_buf[s, 0, :, cols] = val.astype(out_buf.dtype)
        for _ in ffn:
            pass
        return tuple(y)

    y = lax.fori_loop(
        0, n_fin, finish, tuple(jnp.zeros((8, _LANES), _F32) for _ in range(n_blk)))

    order = picked >> (seq.bit_length() - 1)
    bits = jnp.where(order >= 0x8000, order - 0x8000, 0xFFFF - order)
    r_sel = jax.nn.sigmoid(pltpu.bitcast(bits << 16, _F32))
    tokens = [tok_buf[i] for i in range(_TOP_C)]
    out_copy((pl.ds(0, n_seg), pl.ds(1, 3)), 0).wait()
    for j in range(n_fin - 1):
        first_copy(j).wait()
    for i, tok in enumerate(tokens):
        at = pl.ds(tok, 1)
        rest = 1.0 - g_buf[at, :]
        acc_buf[at, :] += jnp.concatenate([rest * (yn * r_sel)[i:i + 1] for yn in y], axis=1)
    for tok in tokens:
        rows = pl.ds(pl.multiple_of((tok >> 3) * 8, 8), 8)
        out_buf[tok >> 5, (tok >> 3) & 3] = acc_buf[rows, :].astype(out_buf.dtype)
    first_copy(n_fin - 1).start()
    patches = []
    for i, tok in enumerate(tokens):
        new = True
        for other in tokens[:i]:
            new = new & ((tok >> 3) != (other >> 3))
        leading = ((tok >> 3) & 3) == 0
        at = (pl.ds(tok >> 5, 1), pl.ds((tok >> 3) & 3, 1))
        patches.append((new & ~leading, out_copy(at, 0)))
        patches.append((new & leading, out_copy(
            at + (pl.ds(0, 8), pl.ds(0, d_model - 2 * _LANES)), 0)))
    for needed, c in patches:
        pl.when(needed)(c.start)
    for needed, c in patches:
        pl.when(needed)(c.wait)
    first_copy(n_fin - 1).wait()


@functools.partial(jax.jit, static_argnames=("A_seg_len",))
def pallas_gated_mix__memory_aug_recurrent_mem_tr__moe_arch_mod__prompt_kernel(
    A_x, A_mem0, A_Wq, A_Wk, A_Wv, A_Wo, A_seg_len,
    B_x, B_w_r, B_w_gate, B_w_up, B_w_down, gate_w,
):
    del B_x
    batch, seq, d_model = A_x.shape
    _, n_heads, d_head = A_Wq.shape
    d_ff = B_w_gate.shape[1]
    assert (batch, A_seg_len, A_mem0.shape[1]) == (1, 32, 8)
    assert (d_model, n_heads, d_head) == (1024, 32, _LANES) and d_ff % 512 == 0
    assert seq >= 1024 and seq & (seq - 1) == 0
    n_seg = seq // A_seg_len
    n_blk, f_blk = d_model // _LANES, d_ff // _LANES

    hbm = pl.BlockSpec(memory_space=pl.ANY)
    dma = pltpu.SemaphoreType.DMA
    out = pl.pallas_call(
        functools.partial(_kernel, n_seg=n_seg, n_heads=n_heads, d_model=d_model,
                          d_ff=d_ff, scale=d_head ** -0.5),
        out_shape=jax.ShapeDtypeStruct((n_seg, 4, 8, d_model), A_x.dtype),
        in_specs=[hbm] * 11,
        out_specs=hbm,
        scratch_shapes=[
            pltpu.VMEM((n_seg, 4, 8, d_model), A_x.dtype),
            pltpu.VMEM((n_seg * 4, d_model), _U32),
            pltpu.VMEM((2, 3, d_model + 16, _LANES), _U32),
            pltpu.VMEM((3, n_heads, d_model // 2, _LANES), _U32),
            pltpu.VMEM((n_blk, n_heads * d_head // 2, _LANES), _U32),
            pltpu.VMEM((f_blk, d_model // 2, _LANES), _U32),
            pltpu.VMEM((f_blk, d_model // 2, _LANES), _U32),
            pltpu.VMEM((n_blk, d_ff // 2, _LANES), _U32),
            pltpu.VMEM((3, n_heads, n_seg * 8, _LANES), _F32),
            pltpu.VMEM((n_heads, n_seg * 4, _LANES), _U32),
            pltpu.VMEM((seq, d_model), _F32),
            pltpu.VMEM((seq, _LANES), _F32),
            pltpu.VMEM((n_seg, 4, 8, d_model), A_x.dtype),
            pltpu.VMEM((8, d_model), A_mem0.dtype),
            pltpu.VMEM((n_blk, _LANES), B_w_r.dtype),
            pltpu.VMEM((n_blk, _LANES), gate_w.dtype),
            pltpu.SMEM((n_seg // 4,), jnp.int32),
            dma((2, 3)), dma((2,)), dma((2,)), dma((1,)), dma((1,)), dma((1,)), dma((2,)),
        ],
        compiler_params=pltpu.CompilerParams(
            vmem_limit_bytes=120 * 2**20,
            disable_bounds_checks=True,
            flags={"XLA_TPU_EVENLY_DISTRIBUTE_CRITICAL_NODES": True},
        ),
        name="gated_rmt_mod",
    )(
        A_x.reshape(n_seg, 4, 8, d_model),
        A_mem0.reshape(8, d_model),
        A_Wq, A_Wk, A_Wv,
        A_Wo.reshape(n_heads * d_head, d_model),
        B_w_r.reshape(n_blk, _LANES), gate_w.reshape(n_blk, _LANES),
        B_w_gate, B_w_up, B_w_down,
    )
    return out.reshape(batch, seq, d_model)
```
